```python
import os as _os
_os.environ.setdefault("JAX_PLATFORMS", "cpu")
import jax
import jax.numpy as jnp

def _softmax(x, axis=-1):
    return jax.nn.softmax(x, axis=axis)
def _gelu(x):
    return jax.nn.gelu(x, approximate=True)
def _silu(x):
    return jax.nn.silu(x)
def _sigmoid(x):
    return jax.nn.sigmoid(x)
def _layernorm(x, axis=-1, eps=1e-5):
    m = jnp.mean(x, axis=axis, keepdims=True)
    v = jnp.var(x, axis=axis, keepdims=True)
    return (x - m) / jnp.sqrt(v + eps)
def _scatter_add(tgt, idx, src, axis=0):
    return tgt.at[idx].add(src)
def _segment_sum(src, seg, n):
    return jax.ops.segment_sum(src, seg, n)
class _Rng:
    def __init__(self, key):
        self._k = key
    def _next(self):
        self._k, sub = jax.random.split(self._k)
        return sub
    def normal(self, shape):
        return jax.random.normal(self._next(), shape, dtype=jnp.bfloat16)
    def randint(self, lo, hi, shape):
        return jax.random.randint(self._next(), shape, lo, hi, dtype=jnp.int32)
    def uniform(self, shape, lo=0.0, hi=1.0):
        return jax.random.uniform(self._next(), shape, jnp.bfloat16, lo, hi)
    def permutation(self, n):
        return jax.random.permutation(self._next(), n)


kernel_name = 'standalone__gqa_block_cached__near_ridge'

def setup_inputs():
    _rng = _Rng(jax.random.key(int.from_bytes(__import__("os").urandom(4), "little")))
    _w = (lambda a: (lambda t: t.astype(jnp.bfloat16) if jnp.issubdtype(t.dtype, jnp.floating) else t)(jnp.asarray(a)))
    B, Sq, D = 8, 144, 448
    Hq, Hkv, Sk, Dh = 16, 8, 2048, 256
    assert Hq % Hkv == 0, (Hq, Hkv)
    return {
        "x": _w((lambda *s: _rng.normal(s) * 0.8)(B, Sq, D)),
        "k_cache": _w((lambda *s: _rng.normal(s) * 0.8)(B, Hkv, Sk, Dh)),
        "v_cache": _w((lambda *s: _rng.normal(s) * 0.05)(B, Hkv, Sk, Dh)),
        "wq": _w((lambda *s: _rng.normal(s) * 0.8)(D, Hq * Dh) * (D ** -0.5)),
        "wo": _w((lambda *s: _rng.normal(s) * 0.05)(Hq * Dh, D) * ((Hq * Dh) ** -0.5)),
    }

def reference(x, k_cache, v_cache, wq, wo):
    B, Sq, D = x.shape
    Hq, Dh = 16, 256
    Hkv = k_cache.shape[1]
    rep = Hq // Hkv
    q = (lambda x, *d: x.transpose(*d))((x @ wq).reshape(B, Sq, Hq, Dh), 0, 2, 1, 3)
    k = jnp.repeat(k_cache, rep, axis=1)
    v = jnp.repeat(v_cache, rep, axis=1)
    scores = jnp.einsum("bhqd,bhkd->bhqk", q, k) * (Dh ** -0.5)
    p = _softmax(scores, axis=-1)
    o = jnp.einsum("bhqk,bhkd->bhqd", p, v)
    return (lambda x, *d: x.transpose(*d))(o, 0, 2, 1, 3).reshape(B, Sq, Hq * Dh) @ wo
```

```python
import functools
import jax, jax.numpy as jnp
from jax import lax
import jax.experimental.pallas as pl
import jax.experimental.pallas.tpu as pltpu

NT = (((1,), (1,)), ((), ()))
LOG2E = 1.4426950408889634
bf16 = jnp.bfloat16
f32 = jnp.float32

class _Null:
    def __enter__(self): return self
    def __exit__(self, *a): return False

def make(U=4, vmem=120, RC=16, X0=3, hsec=(1, 4), ochunks=(384, 384, 256, 128), scopes=False, nobc=True, gate=True):
    scope = (lambda n: jax.named_scope(n)) if scopes else (lambda n: _Null())
    def kernel_fn(x, k_cache, v_cache, wq, wo):
        B, Sq, D = x.shape
        _, Hkv, Sk, Dh = k_cache.shape
        Hq = wq.shape[1] // Dh
        rep = Hq // Hkv
        G = rep * Dh
        M = rep * Sq
        R = B * Sq
        scale = Dh ** -0.5 * LOG2E
        NU = B * Hkv
        NB = NU // U
        BPB = Hkv // U
        assert sum(ochunks) == R
        NO = len(ochunks)
        ostart = [sum(ochunks[:i]) for i in range(NO)]
        x2 = x.reshape(R, D)
        k2 = k_cache.reshape(NB, U, Sk, Dh)
        v2 = v_cache.reshape(NB, U, Sk, Dh)
        woT = wo.T
        hb = (0,) + tuple(hsec) + (Hkv,)
        NW = len(hb) - 1
        SK, SV, SX, SW, SWO, SO = 0, 2, 4, 6, 6 + NW, 7 + NW
        NSEM = SO + NO

        def body(x_hbm, k_hbm, v_hbm, wq_hbm, wo_hbm, o_hbm,
                 xbuf, wqbuf, wobuf, kbuf, vbuf, q_u32, ou_all, l_all, obuf,
                 sem, z_ref, *rest):
            s_refs = rest[:U]
            m_refs = rest[U:2 * U]
            p_ref = rest[2 * U].bitcast(bf16)
            q_all = q_u32.bitcast(bf16)
            z_ref[0] = 0

            def k_copy(blk, slot):
                return pltpu.make_async_copy(k_hbm.at[blk], kbuf.at[slot], sem.at[SK + slot])

            def v_copy(blk, slot):
                return pltpu.make_async_copy(v_hbm.at[blk], vbuf.at[slot], sem.at[SV + slot])

            def wq_copy(i):
                c0, n = hb[i] * G, (hb[i + 1] - hb[i]) * G
                return pltpu.make_async_copy(wq_hbm.at[:, pl.ds(c0, n)], wqbuf.at[:, pl.ds(c0, n)], sem.at[SW + i])

            def x_copy(c):
                r0, n = (0, X0 * Sq) if c == 0 else (X0 * Sq, R - X0 * Sq)
                return pltpu.make_async_copy(x_hbm.at[pl.ds(r0, n)], xbuf.at[pl.ds(r0, n)], sem.at[SX + c])

            def o_copy(i):
                return pltpu.make_async_copy(obuf.at[pl.ds(ostart[i], ochunks[i])],
                                             o_hbm.at[pl.ds(ostart[i], ochunks[i])], sem.at[SO + i])

            wo_cp = pltpu.make_async_copy(wo_hbm, wobuf, sem.at[SWO])
            x_copy(0).start()
            wq_copy(0).start()
            x_copy(1).start()
            for i in range(1, NW):
                wq_copy(i).start()
            k_copy(0, 0).start()
            v_copy(0, 0).start()
            k_copy(1, 1).start()
            v_copy(1, 1).start()
            wo_cp.start(priority=1)

            def qproj_rows(h, b0, nb):
                q = jnp.dot(xbuf[b0 * Sq:(b0 + nb) * Sq, :], wqbuf[:, h * G:(h + 1) * G], preferred_element_type=f32)
                q = q * scale
                for b in range(nb):
                    qd = q_all.at[(b0 + b) * Hkv + h]
                    for r in range(rep):
                        qd[r * Sq:(r + 1) * Sq, :] = q[b * Sq:(b + 1) * Sq, r * Dh:(r + 1) * Dh].astype(bf16)

            def qk(unit, slot, j):
                s = lax.dot_general(q_all[unit], kbuf[slot, j], NT, preferred_element_type=f32)
                s_refs[j][...] = s
                m_refs[j][...] = jnp.broadcast_to(jnp.max(s, axis=-1, keepdims=True), (M, 128))

            def sm(b, h, j, store):
                ps = []
                for r0 in range(0, M, RC):
                    s = s_refs[j][r0:r0 + RC, :]
                    m = m_refs[j][r0:r0 + RC, :]
                    p = jnp.exp2(s - jnp.concatenate([m] * (Sk // 128), axis=1))
                    lp = p[:, 0:128]
                    for c in range(1, Sk // 128):
                        lp = lp + p[:, c * 128:(c + 1) * 128]
                    row = b * Sq + r0 % Sq
                    if not isinstance(row, int):
                        row = pl.multiple_of(row, RC)
                    l_all[h * rep + r0 // Sq, pl.ds(row, RC), :] = lp
                    if store:
                        p_ref.at[0][r0:r0 + RC, :] = p.astype(bf16)
                    else:
                        ps.append(p)
                if not store:
                    return jnp.concatenate(ps, axis=0).astype(bf16)

            def pv(b, h, p, slot, j):
                o = jnp.dot(p, vbuf[slot, j], preferred_element_type=f32)
                row = b * Sq
                if not isinstance(row, int):
                    row = pl.multiple_of(row, 16)
                for r in range(rep):
                    ou_all[h * rep + r, pl.ds(row, Sq), :] = o[r * Sq:(r + 1) * Sq]

            with scope('q0'):
                x_copy(0).wait()
                wq_copy(0).wait()
                for h in range(hb[0], hb[1]):
                    qproj_rows(h, 0, X0)
            with scope('q1'):
                x_copy(1).wait()
                for h in range(hb[0], hb[1]):
                    qproj_rows(h, X0, B - X0)
            for i in range(1, NW):
                with scope('q%d' % (i + 1)):
                    wq_copy(i).wait()
                    if i == NW - 1:
                        k_copy(0, 0).wait()
                    for h in range(hb[i], hb[i + 1]):
                        qproj_rows(h, 0, B)
                    if i == NW - 1:
                        for j in range(U):
                            qk(j, 0, j)
                        k_copy(2, 0).start()

            def block(t, c):
                slot = t & 1
                v_copy(0, slot).wait()
                k_copy(0, 1 - slot).wait()
                z = z_ref[0]
                b = t // BPB
                h0 = lax.rem(t, BPB) * U
                for j in range(U - 1):
                    pv(b, h0 + j, sm(b, h0 + j, j, False), slot, j)
                    qk((t + 1) * U + j, 1 - slot, j)
                j = U - 1
                sm(b, h0 + j, j, True)
                qk((t + 1) * U + j, 1 - slot, j)
                pv(b, h0 + j, p_ref[z], slot, j)

                @pl.when(t + 3 < NB)
                def _():
                    k_copy(t + 3, 1 - slot).start()

                @pl.when(t + 2 < NB)
                def _():
                    v_copy(t + 2, slot).start()
                return c

            with scope('main'):
                lax.fori_loop(0, NB - 1, block, 0)

            def norm(hq, row0, n, tok):
                lp = l_all[hq, row0:row0 + n, :]
                if tok is not None:
                    lp = lp + jnp.concatenate([tok] * (n // 8), axis=0)
                l = jnp.sum(lp, axis=-1, keepdims=True)
                r0 = pl.reciprocal(l, approx=True)
                li = r0 * (2.0 - l * r0)
                return (ou_all[hq, row0:row0 + n, :] * li).astype(bf16)

            toks = {}
            def oproj(i):
                row0, n = ostart[i], ochunks[i]
                acc = None
                for h in range(Hkv):
                    tok = toks.get(i - 1 if h >= Hkv // 2 else i - 2) if gate else None
                    o = jnp.concatenate([norm(h * rep + r, row0, n, tok) for r in range(rep)], axis=1)
                    part = lax.dot_general(wobuf[:, h * G:(h + 1) * G], o, NT, preferred_element_type=f32)
                    acc = part if acc is None else acc + part
                acct = acc.T
                toks[i] = jnp.where(z_ref[0] != 0, acct[n - 8:n, 256:384], 0.0)
                obuf[row0:row0 + n, :] = acct.astype(obuf.dtype)
                o_copy(i).start()

            with scope('last'):
                t = NB - 1
                v_copy(0, t % 2).wait()
                wo_cp.wait()
                for j in range(U):
                    b, h = t // BPB, (t % BPB) * U + j
                    pv(b, h, sm(b, h, j, False), t % 2, j)
                for i in range(NO):
                    oproj(i)
            with scope('owait'):
                for i in range(NO):
                    o_copy(i).wait()

        anyspec = pl.BlockSpec(memory_space=pl.ANY)
        out = pl.pallas_call(
            body,
            in_specs=[anyspec] * 5,
            out_specs=anyspec,
            out_shape=jax.ShapeDtypeStruct((R, D), x.dtype),
            scratch_shapes=[
                pltpu.VMEM((R, D), bf16),
                pltpu.VMEM((D, Hkv * G), bf16),
                pltpu.VMEM((D, Hkv * G), bf16),
                pltpu.VMEM((2, U, Sk, Dh), bf16),
                pltpu.VMEM((2, U, Sk, Dh), bf16),
                pltpu.VMEM((NU, M // 2, Dh), jnp.uint32),
                pltpu.VMEM((Hq, R, Dh), f32),
                pltpu.VMEM((Hq, R, 128), f32),
                pltpu.VMEM((R, D), bf16),
                pltpu.SemaphoreType.DMA((NSEM,)),
                pltpu.SMEM((1,), jnp.int32),
            ] + [pltpu.VMEM((M, Sk), f32)] * U + [pltpu.VMEM((M, 128), f32)] * U
              + [pltpu.VMEM((1, M // 2, Sk), jnp.uint32)],
            compiler_params=pltpu.CompilerParams(vmem_limit_bytes=vmem * 1024 * 1024, disable_bounds_checks=nobc),
        )(x2, k2, v2, wq, woT)
        return out.reshape(B, Sq, D)
    return kernel_fn


@jax.jit
def pallas_standalone__gqa_block_cached__near_ridge_kernel(x, k_cache, v_cache, wq, wo):
    return make()(x, k_cache, v_cache, wq, wo)
```

```python
import functools
import jax, jax.numpy as jnp
from jax import lax
import jax.experimental.pallas as pl
import jax.experimental.pallas.tpu as pltpu

NT = (((1,), (1,)), ((), ()))
LOG2E = 1.4426950408889634
bf16 = jnp.bfloat16
f32 = jnp.float32

class _Null:
    def __enter__(self): return self
    def __exit__(self, *a): return False

def make(U=4, vmem=120, secs=((2, 2), (5, 2), (8, 4), (8, 10), (8, 16)),
         ochunks=(256, 256, 256, 256, 128), oo=(2, 5, 1, 3, 6, 4, 7), gg=2, oz=(1, None, 3, 4, None, 6, 7), lgate=6, scopes=False, gh=6, NTC=256,
         mo=(1, 4, 5, 7, 2, 3, 6), spv=True, PW=512, po=(3, 4, 7, 5, 6, 2, 1), tailn=2, cond=True, kz=(0, 1, 1, 0, 0, 1, 0), vz=(0, 1, 2, 3, 4, 5, 6)):
    scope = (lambda n: jax.named_scope(n)) if scopes else (lambda n: _Null())
    def kernel_fn(x, k_cache, v_cache, wq, wo):
        B, Sq, D = x.shape
        _, Hkv, Sk, Dh = k_cache.shape
        Hq = wq.shape[1] // Dh
        rep = Hq // Hkv
        G = rep * Dh
        M = rep * Sq
        R = B * Sq
        H = Dh // 2
        scale = Dh ** -0.5 * LOG2E
        NU = B * Hkv
        NB = NU // U
        BPB = Hkv // U
        assert sum(ochunks) == R and secs[-1] == (B, Hq) and rep == 2 and H == 128
        NO = len(ochunks)
        NS = len(secs)
        ostart = [sum(ochunks[:i]) for i in range(NO)]
        x2 = x.reshape(R, D)
        k2 = k_cache.reshape(NB, U, Sk, Dh)
        v2 = v_cache.reshape(NB, U, Sk, Dh)
        woT = wo.T
        SK, SV, SWO, SO, SX = 0, 2, 4, 5, 6
        NSEM = SX + NS
        prev = ((0, 0),) + tuple(secs[:-1])

        def body(x_hbm, k_hbm, v_hbm, wq_hbm, wo_hbm, o_hbm,
                 xbuf, wqbuf, wobuf, kbuf, vbuf, q_u32, ou_all, obuf,
                 sem, z_ref, *rest):
            s_refs = rest[:U]
            m_refs = rest[U:2 * U]
            q_all = q_u32.bitcast(bf16)
            for i in range(16):
                z_ref[i] = 0

            def k_copy(blk, slot, j=None):
                if j is None:
                    return pltpu.make_async_copy(k_hbm.at[blk], kbuf.at[slot], sem.at[SK + slot])
                return pltpu.make_async_copy(k_hbm.at[blk, j], kbuf.at[slot, j], sem.at[SK + slot])

            def v_copy(blk, slot, j=None):
                if j is None:
                    return pltpu.make_async_copy(v_hbm.at[blk], vbuf.at[slot], sem.at[SV + slot])
                return pltpu.make_async_copy(v_hbm.at[blk, j], vbuf.at[slot, j], sem.at[SV + slot])

            def sec_copies(i):
                (a0, c0), (a1, c1) = prev[i], secs[i]
                cps = []
                if a1 > a0:
                    sl = pl.ds(a0 * Sq, (a1 - a0) * Sq)
                    cps.append(pltpu.make_async_copy(x_hbm.at[sl], xbuf.at[sl], sem.at[SX + i]))
                if c1 > c0:
                    sl = pl.ds(c0 * Dh, (c1 - c0) * Dh)
                    cps.append(pltpu.make_async_copy(wq_hbm.at[:, sl], wqbuf.at[:, sl], sem.at[SX + i]))
                return cps

            def o_copy(i):
                return pltpu.make_async_copy(obuf.at[pl.ds(ostart[i], ochunks[i])],
                                             o_hbm.at[pl.ds(ostart[i], ochunks[i])], sem.at[SO])

            wo_cp = pltpu.make_async_copy(wo_hbm, wobuf, sem.at[SWO])
            for i in range(NS):
                for cp in sec_copies(i):
                    cp.start()
            k_copy(0, 0).start()
            v_copy(0, 0).start()
            k_copy(1, 1).start()
            v_copy(1, 1).start()
            wo_cp.start(priority=1)

            def qproj(b0, b1, c0, c1):
                if b1 <= b0:
                    return
                for cc in range(c0, c1, rep):
                    q = jnp.dot(xbuf[b0 * Sq:b1 * Sq, :], wqbuf[:, cc * Dh:(cc + rep) * Dh], preferred_element_type=f32)
                    q = q * scale
                    for b in range(b0, b1):
                        qd = q_all.at[b * Hkv + cc // rep]
                        qb = q[(b - b0) * Sq:(b - b0 + 1) * Sq]
                        a11, a12, a21, a22 = [qb[:, i * H:(i + 1) * H] for i in range(4)]
                        ops = [a11 + a22, a21 + a22, a11, a22, a11 + a12, a21 - a11, a12 - a22]
                        for i, a in enumerate(ops):
                            qd[:, i * H:(i + 1) * H] = a.astype(bf16)

            def rhs_ops(b11, b12, b21, b22):
                f = lambda t, i: t(i).astype(f32)
                return {1: lambda: (f(b11, 1) + f(b22, 1)).astype(bf16), 2: lambda: b11(2),
                        3: lambda: (f(b12, 3) - f(b22, 3)).astype(bf16),
                        4: lambda: (f(b21, 4) - f(b11, 4)).astype(bf16), 5: lambda: b22(5),
                        6: lambda: (f(b11, 6) + f(b12, 6)).astype(bf16),
                        7: lambda: (f(b21, 7) + f(b22, 7)).astype(bf16)}

            def combine(mm):
                return ((mm[1] + mm[4]) + (mm[7] - mm[5]), mm[3] + mm[5], mm[2] + mm[4],
                        (mm[1] - mm[2]) + (mm[3] + mm[6]))

            def finish_m(mp):
                m = jnp.max(mp, axis=-1, keepdims=True)
                if spv and cond:
                    m = m + jnp.log2(jnp.sum(jnp.exp2(mp - m), axis=-1, keepdims=True))
                return jnp.broadcast_to(m, mp.shape)

            def recip(l):
                r0 = pl.reciprocal(l, approx=True)
                return r0 * (2.0 - l * r0)

            def qk(unit, slot, j):
                qd = q_all.at[unit]
                kv = {zi: kbuf.at[slot + z_ref[zi], j] for zi in set(kz)}
                kd = {i: kv[kz[i - 1]] for i in range(1, 8)}
                ma = mb = None
                for c0 in range(0, Sk, 2 * H):
                    w = rhs_ops(lambda i: kd[i][c0:c0 + H, 0:H], lambda i: kd[i][c0 + H:c0 + 2 * H, 0:H],
                                lambda i: kd[i][c0:c0 + H, H:Dh], lambda i: kd[i][c0 + H:c0 + 2 * H, H:Dh])
                    mm = {}
                    for i in mo:
                        mm[i] = lax.dot_general(qd[:, (i - 1) * H:i * H], w[i](), NT, preferred_element_type=f32)
                    c11, c12, c21, c22 = combine(mm)
                    s_refs[j][0:Sq, c0:c0 + H] = c11
                    s_refs[j][0:Sq, c0 + H:c0 + 2 * H] = c12
                    s_refs[j][Sq:M, c0:c0 + H] = c21
                    s_refs[j][Sq:M, c0 + H:c0 + 2 * H] = c22
                    ta = jnp.maximum(c11, c12)
                    tb = jnp.maximum(c21, c22)
                    ma = ta if ma is None else jnp.maximum(ma, ta)
                    mb = tb if mb is None else jnp.maximum(mb, tb)
                m_refs[j][0:Sq, :] = finish_m(ma)
                m_refs[j][Sq:M, :] = finish_m(mb)

            def smpv(b, h, slot, j, mid=None):
                row = b * Sq
                if not isinstance(row, int):
                    row = pl.multiple_of(row, 16)
                vv = {zi: vbuf.at[slot + z_ref[zi], j] for zi in set(vz)}
                vd = {i: vv[vz[i - 1]] for i in range(1, 8)}

                def pblk(r0, c0):
                    m = m_refs[j][r0:r0 + Sq, :]
                    return jnp.exp2(s_refs[j][r0:r0 + Sq, c0:c0 + PW] - jnp.concatenate([m] * (PW // 128), axis=1))

                def fold(acc, t):
                    for c in range(PW // 128):
                        u = t[:, c * 128:(c + 1) * 128]
                        acc = u if acc is None else acc + u
                    return acc

                mm = {}
                la = lb = None
                for c0 in range(0, Sk, 2 * PW):
                    a11, a12, a21, a22 = pblk(0, c0), pblk(0, c0 + PW), pblk(Sq, c0), pblk(Sq, c0 + PW)
                    sa, sb = a11 + a12, a21 + a22
                    la, lb = fold(la, sa), fold(lb, sb)
                    a = {1: lambda: a11 + a22, 2: lambda: sb, 3: lambda: a11, 4: lambda: a22,
                         5: lambda: sa, 6: lambda: a21 - a11, 7: lambda: a12 - a22}
                    w = rhs_ops(lambda i: vd[i][c0:c0 + PW, 0:H], lambda i: vd[i][c0:c0 + PW, H:Dh],
                                lambda i: vd[i][c0 + PW:c0 + 2 * PW, 0:H], lambda i: vd[i][c0 + PW:c0 + 2 * PW, H:Dh])
                    for n, i in enumerate(po):
                        if mid is not None and c0 + 2 * PW == Sk and n == 7 - tailn:
                            mid()
                        t = jnp.dot(a[i]().astype(bf16), w[i](), preferred_element_type=f32)
                        mm[i] = t if i not in mm else mm[i] + t
                c11, c12, c21, c22 = combine(mm)
                never = z_ref[0] != 0
                ia = recip(jnp.sum(jnp.where(never, mm[lgate], la), axis=-1, keepdims=True))
                ib = recip(jnp.sum(jnp.where(never, mm[lgate], lb), axis=-1, keepdims=True))
                ou_all[h * rep, pl.ds(row, Sq), 0:H] = c11 * ia
                ou_all[h * rep, pl.ds(row, Sq), H:Dh] = c12 * ia
                ou_all[h * rep + 1, pl.ds(row, Sq), 0:H] = c21 * ib
                ou_all[h * rep + 1, pl.ds(row, Sq), H:Dh] = c22 * ib

            for i in range(NS):
                with scope('q%d' % i):
                    (a0, c0), (a1, c1) = prev[i], secs[i]
                    for cp in sec_copies(i):
                        cp.wait()
                    if i == NS - 1:
                        k_copy(0, 0).wait()
                        for j in range(U):
                            qk(j, 0, j)
                        k_copy(2, 0).start()
                    qproj(a0, a1, 0, c0)
                    qproj(0, a1, c0, c1)

            def block(t, c):
                slot = t & 1
                v_copy(t, slot).wait()
                k_copy(t + 1, 1 - slot).wait()
                b = t // BPB
                h0 = lax.rem(t, BPB) * U
                for j in range(U):
                    def do_qk():
                        qk((t + 1) * U + j, 1 - slot, j)

                        @pl.when(t + 3 < NB)
                        def _():
                            k_copy(t + 3, 1 - slot, j).start()

                    smpv(b, h0 + j, slot, j, do_qk if j == U - 1 else None)

                    @pl.when(t + 2 < NB)
                    def _():
                        v_copy(t + 2, slot, j).start()

                    if j != U - 1:
                        do_qk()
                return c

            def block2(t, c):
                with scope('blk'):
                    return block(t, c)
            with scope('main'):
                lax.fori_loop(0, NB - 1, block2, 0)

            def finish_chunk(i):
                o_copy(i).start()
                z = z_ref[0]
                tk = obuf[pl.ds(pl.multiple_of(ostart[i] + z, 16), 16), 0:128].astype(f32)[0:8]
                toks[i] = jnp.where(z != 0, tk, 0.0)

            toks = {}
            wops = {}
            DH = D // 2

            def gated(t, tok):
                if tok is None:
                    return t
                top = jnp.concatenate([t[0:8, 0:128] + tok, t[0:8, 128:]], axis=1)
                return jnp.concatenate([top, t[8:]], axis=0)

            def oproj_strassen(i):
                row0 = ostart[i]
                mm = {}
                for g in range(Hkv // 2):
                    tok = toks.get(i - 1) if g == gg else None
                    k1, k2 = 2 * g * G, (2 * g + 1) * G
                    f = lambda r, k, zi: wobuf[pl.ds(pl.multiple_of(r * DH + z_ref[zi], 16), DH), k:k + G]
                    ff = lambda r, k, zi: f(r, k, zi).astype(f32)
                    if g not in wops:
                        wops[g] = {1: (ff(0, k1, 1) + ff(1, k2, 1)).astype(bf16), 2: (ff(1, k1, 2) + ff(1, k2, 2)).astype(bf16),
                                   5: (ff(0, k1, 5) + ff(0, k2, 5)).astype(bf16),
                                   6: (ff(1, k1, 6) - ff(0, k1, 6)).astype(bf16), 7: (ff(0, k2, 7) - ff(1, k2, 7)).astype(bf16)}
                    a = dict(wops[g])
                    a[3], a[4] = f(0, k1, 8 + i), f(1, k2, 8 + i)

                    def ob(kk, tt, p):
                        zz = 0 if oz[p - 1] is None else z_ref[oz[p - 1]]
                        return jnp.concatenate(
                            [ou_all[4 * g + 2 * kk + r + zz, row0 + tt * 128:row0 + (tt + 1) * 128, :]
                             for r in range(rep)], axis=1)
                    w = {1: lambda: ob(0, 0, 1) + ob(1, 1, 1), 2: lambda: gated(ob(0, 0, 2), tok),
                         3: lambda: ob(0, 1, 3) - ob(1, 1, 3),
                         4: lambda: ob(1, 0, 4) - ob(0, 0, 4), 5: lambda: ob(1, 1, 5), 6: lambda: ob(0, 0, 6) + ob(0, 1, 6),
                         7: lambda: ob(1, 0, 7) + ob(1, 1, 7)}
                    for p in oo:
                        t = lax.dot_general(a[p], w[p]().astype(bf16), NT, preferred_element_type=f32)
                        mm[p] = t if p not in mm else mm[p] + t
                c11, c12, c21, c22 = combine(mm)
                obuf[row0:row0 + 128, :] = jnp.concatenate([c11, c21], axis=0).T.astype(obuf.dtype)
                obuf[row0 + 128:row0 + 256, :] = jnp.concatenate([c12, c22], axis=0).T.astype(obuf.dtype)
                finish_chunk(i)

            def oproj(i):
                row0, n = ostart[i], ochunks[i]
                if n == 256:
                    return oproj_strassen(i)
                acc = None
                c0 = NTC if i == NO - 1 else 0
                os_ = []
                for h in range(Hkv):
                    tok = toks.get(i - 1) if h == gh else None
                    o = jnp.concatenate([ou_all[h * rep + r, row0:row0 + n, :] for r in range(rep)], axis=1)
                    o = gated(o, tok).astype(bf16)
                    os_.append(o)
                    part = lax.dot_general(wobuf[c0:, h * G:(h + 1) * G], o, NT, preferred_element_type=f32)
                    acc = part if acc is None else acc + part
                obuf[row0:row0 + n, c0:] = acc.T.astype(obuf.dtype)
                if c0:
                    o = jnp.concatenate(os_, axis=1)
                    obuf[row0:row0 + n, 0:c0] = lax.dot_general(
                        o, wobuf[0:c0, :], NT, preferred_element_type=f32).astype(obuf.dtype)
                finish_chunk(i)

            with scope('last'):
                t = NB - 1
                v_copy(t, t % 2).wait()
                wo_cp.wait()
                for j in range(U):
                    smpv(t // BPB, (t % BPB) * U + j, t % 2, j)
                for i in range(NO):
                    oproj(i)
            with scope('owait'):
                for i in range(NO):
                    o_copy(i).wait()

        anyspec = pl.BlockSpec(memory_space=pl.ANY)
        out = pl.pallas_call(
            body,
            in_specs=[anyspec] * 5,
            out_specs=anyspec,
            out_shape=jax.ShapeDtypeStruct((R, D), x.dtype),
            scratch_shapes=[
                pltpu.VMEM((R, D), bf16),
                pltpu.VMEM((D, Hkv * G), bf16),
                pltpu.VMEM((D, Hkv * G), bf16),
                pltpu.VMEM((2, U, Sk, Dh), bf16),
                pltpu.VMEM((2, U, Sk, Dh), bf16),
                pltpu.VMEM((NU, Sq // 2, 7 * H), jnp.uint32),
                pltpu.VMEM((Hq, R, Dh), f32),
                pltpu.VMEM((R, D), bf16),
                pltpu.SemaphoreType.DMA((NSEM,)),
                pltpu.SMEM((16,), jnp.int32),
            ] + [pltpu.VMEM((M, Sk), f32)] * U + [pltpu.VMEM((M, 128), f32)] * U,
            compiler_params=pltpu.CompilerParams(vmem_limit_bytes=vmem * 1024 * 1024, disable_bounds_checks=True,
                                                 disable_semaphore_checks=True),
        )(x2, k2, v2, wq, woT)
        return out.reshape(B, Sq, D)
    return kernel_fn


@jax.jit
def pallas_standalone__gqa_block_cached__near_ridge_kernel(x, k_cache, v_cache, wq, wo):
    return make()(x, k_cache, v_cache, wq, wo)
```

```python
import jax
import jax.numpy as jnp
from jax import lax
import jax.experimental.pallas as pl
import jax.experimental.pallas.tpu as pltpu

_NT = (((1,), (1,)), ((), ()))
_LOG2E = 1.4426950408889634
_BF16 = jnp.bfloat16
_F32 = jnp.float32

_U = 4
_T = 128
_SECTIONS = ((2, 2), (5, 2), (8, 4), (8, 10), (8, 16))
_Q_STRASSEN_FROM = 2
_O_CHUNKS = (256, 256, 256, 256, 128)
_PW = 512
_Q_ORDER = (2, 4, 1, 6, 3, 5, 7)
_QK_ORDER = (5, 3, 1, 7, 4, 2, 6)
_PV_ORDER = (3, 4, 7, 5, 6, 2, 1)
_O_ORDER = (2, 5, 1, 3, 6, 4, 7)
_K_Z = (0, 1, 0, 1, 0, 1, 0)
_V_Z = (0, 1, None, 3, 4, 5, 6)
_O_Z = (1, None, 3, 4, None, 6, 7)
_NZ = 16


def _combine(m):
    return ((m[1] + m[4]) + (m[7] - m[5]), m[3] + m[5], m[2] + m[4], (m[1] - m[2]) + (m[3] + m[6]))


def _rhs_operands(b11, b12, b21, b22):
    f = lambda b, i: b(i).astype(_F32)
    return {1: lambda: (f(b11, 1) + f(b22, 1)).astype(_BF16),
            2: lambda: b11(2),
            3: lambda: (f(b12, 3) - f(b22, 3)).astype(_BF16),
            4: lambda: (f(b21, 4) - f(b11, 4)).astype(_BF16),
            5: lambda: b22(5),
            6: lambda: (f(b11, 6) + f(b12, 6)).astype(_BF16),
            7: lambda: (f(b21, 7) + f(b22, 7)).astype(_BF16)}


def _recip(l):
    r = pl.reciprocal(l, approx=True)
    return r * (2.0 - l * r)


def _softmax_shift(lane_max):
    m = jnp.max(lane_max, axis=-1, keepdims=True)
    m = m + jnp.log2(jnp.sum(jnp.exp2(lane_max - m), axis=-1, keepdims=True))
    return jnp.broadcast_to(m, lane_max.shape)


@jax.jit
def pallas_standalone__gqa_block_cached__near_ridge_kernel(
    x: jax.Array,
    k_cache: jax.Array,
    v_cache: jax.Array,
    wq: jax.Array,
    wo: jax.Array,
):
    B, Sq, D = x.shape
    _, Hkv, Sk, Dh = k_cache.shape
    Hq = wq.shape[1] // Dh
    rep = Hq // Hkv
    U, T, PW = _U, _T, _PW
    G = rep * Dh
    M = rep * Sq
    R = B * Sq
    RH, DH = R // 2, D // 2
    K1 = 2 * T
    K2 = D - K1
    NB = B * Hkv // U
    BPB = Hkv // U
    NS, NO = len(_SECTIONS), len(_O_CHUNKS)
    scale = Dh ** -0.5 * _LOG2E
    assert rep == 2 and Dh == 2 * T and Hkv % U == 0 and Sk % (2 * PW) == 0 and 0 < K2 <= K1
    assert Sq % 16 == 0 and DH % 16 == 0 and sum(_O_CHUNKS) == R and _SECTIONS[-1] == (B, Hq)
    o_start = [sum(_O_CHUNKS[:i]) for i in range(NO)]
    prev_section = ((0, 0),) + _SECTIONS[:-1]
    SEM_K, SEM_V, SEM_WO, SEM_O, SEM_X = 0, 2, 4, 5, 6

    def body(x_hbm, k_hbm, v_hbm, wq_hbm, wo_hbm, o_hbm,
             xbuf, wqbuf, wobuf, kbuf, vbuf, xs_u32, q_u32, o_all, obuf, sem, z_ref, *rest):
        s_refs, m_refs = rest[:U], rest[U:]
        xs = xs_u32.bitcast(_BF16)
        q_all = q_u32.bitcast(_BF16)
        for i in range(_NZ):
            z_ref[i] = 0

        def kv_copy(hbm, buf, sem0, blk, slot, j):
            if j is None:
                return pltpu.make_async_copy(hbm.at[blk], buf.at[slot], sem.at[sem0 + slot])
            return pltpu.make_async_copy(hbm.at[blk, j], buf.at[slot, j], sem.at[sem0 + slot])

        k_copy = lambda blk, slot, j=None: kv_copy(k_hbm, kbuf, SEM_K, blk, slot, j)
        v_copy = lambda blk, slot, j=None: kv_copy(v_hbm, vbuf, SEM_V, blk, slot, j)

        def section_copies(i):
            (a0, c0), (a1, c1) = prev_section[i], _SECTIONS[i]
            cps = []
            if a1 > a0:
                sl = pl.ds(a0 * Sq, (a1 - a0) * Sq)
                cps.append(pltpu.make_async_copy(x_hbm.at[sl], xbuf.at[sl], sem.at[SEM_X + i]))
            if c1 > c0:
                sl = pl.ds(c0 * Dh, (c1 - c0) * Dh)
                cps.append(pltpu.make_async_copy(wq_hbm.at[:, sl], wqbuf.at[:, sl], sem.at[SEM_X + i]))
            return cps

        def out_copy(i):
            sl = pl.ds(o_start[i], _O_CHUNKS[i])
            return pltpu.make_async_copy(obuf.at[sl], o_hbm.at[sl], sem.at[SEM_O])

        wo_copy = pltpu.make_async_copy(wo_hbm, wobuf, sem.at[SEM_WO])

        for i in range(NS):
            for cp in section_copies(i):
                cp.start()
        k_copy(0, 0).start()
        v_copy(0, 0).start()
        k_copy(1, 1).start()
        v_copy(1, 1).start()
        wo_copy.start(priority=1)

        def store_q(b, h, qa, qb):
            a11, a12, a21, a22 = qa[:, 0:T], qa[:, T:Dh], qb[:, 0:T], qb[:, T:Dh]
            ops = (a11 + a22, a21 + a22, a11, a22, a11 + a12, a21 - a11, a12 - a22)
            dst = q_all.at[b * Hkv + h]
            for i, a in enumerate(ops):
                dst[:, i * T:(i + 1) * T] = a.astype(_BF16)

        def qproj(b0, b1, c0, c1):
            if b1 <= b0:
                return
            for c in range(c0, c1, rep):
                q = jnp.dot(xbuf[b0 * Sq:b1 * Sq, :], wqbuf[:, c * Dh:c * Dh + G],
                            preferred_element_type=_F32) * scale
                for b in range(b0, b1):
                    qb = q[(b - b0) * Sq:(b - b0 + 1) * Sq]
                    store_q(b, c // rep, qb[:, 0:Dh], qb[:, Dh:G])

        def prep_x():
            f = lambda r, c0, c1: xbuf[r * RH:(r + 1) * RH, c0:c1].astype(_F32)
            cat = lambda u, v: jnp.concatenate([u, v], axis=1)
            xs[:, 0:K1] = cat(f(0, 0, K2) + f(1, K1, D), f(0, K2, K1)).astype(_BF16)
            xs[:, K1:2 * K1] = cat(f(1, 0, K2) + f(1, K1, D), f(1, K2, K1)).astype(_BF16)
            xs[:, 2 * K1:3 * K1] = (f(1, 0, K1) - f(0, 0, K1)).astype(_BF16)
            xs[:, 3 * K1:3 * K1 + K2] = (f(0, 0, K2) + f(0, K1, D)).astype(_BF16)
            xs[:, 4 * K1:4 * K1 + K2] = (f(0, K1, D) - f(1, K1, D)).astype(_BF16)

        def qproj_strassen(c0, c1):
            for c in range(c0, c1, rep):
                n1, n2 = c * Dh, (c + 1) * Dh
                g = lambda r0, r1, n: wqbuf[r0:r1, n:n + Dh]
                f = lambda r0, r1, n: g(r0, r1, n).astype(_F32)
                cat = lambda u, v: jnp.concatenate([u, v], axis=0)
                a = {1: lambda: xs[:, 0:K1], 2: lambda: xs[:, K1:2 * K1], 3: lambda: xbuf[0:RH, 0:K1],
                     4: lambda: xbuf[RH:R, K1:D], 5: lambda: xs[:, 3 * K1:3 * K1 + K2],
                     6: lambda: xs[:, 2 * K1:3 * K1], 7: lambda: xs[:, 4 * K1:4 * K1 + K2]}
                w = {1: lambda: cat(f(0, K2, n1) + f(K1, D, n2), f(K2, K1, n1)).astype(_BF16),
                     2: lambda: g(0, K1, n1),
                     3: lambda: cat(f(0, K2, n2) - f(K1, D, n2), f(K2, K1, n2)).astype(_BF16),
                     4: lambda: (f(K1, D, n1) - f(0, K2, n1)).astype(_BF16),
                     5: lambda: g(K1, D, n2),
                     6: lambda: (f(0, K1, n1) + f(0, K1, n2)).astype(_BF16),
                     7: lambda: (f(K1, D, n1) + f(K1, D, n2)).astype(_BF16)}
                mm = {}
                for i in _Q_ORDER:
                    mm[i] = jnp.dot(a[i](), w[i](), preferred_element_type=_F32)
                c11, c12, c21, c22 = [t * scale for t in _combine(mm)]
                for b in range(B // 2):
                    rows = slice(b * Sq, (b + 1) * Sq)
                    store_q(b, c // rep, c11[rows], c12[rows])
                    store_q(B // 2 + b, c // rep, c21[rows], c22[rows])

        def store_shift(j, ma, mb, after=None):
            if after is not None:
                never = z_ref[0] != 0
                ma, mb = jnp.where(never, after, ma), jnp.where(never, after, mb)
            m_refs[j][0:Sq, :] = _softmax_shift(ma)
            m_refs[j][Sq:M, :] = _softmax_shift(mb)

        def scores(unit, slot, j, pending=None, defer=False):
            q = q_all.at[unit]
            views = {z: kbuf.at[slot + z_ref[z], j] for z in set(_K_Z)}
            k = lambda i: views[_K_Z[i - 1]]
            ma = mb = None
            for c0 in range(0, Sk, 2 * T):
                c1, c2 = c0 + T, c0 + 2 * T
                w = _rhs_operands(lambda i: k(i)[c0:c1, 0:T], lambda i: k(i)[c1:c2, 0:T],
                                  lambda i: k(i)[c0:c1, T:Dh], lambda i: k(i)[c1:c2, T:Dh])
                mm = {}
                for i in _QK_ORDER:
                    mm[i] = lax.dot_general(q[:, (i - 1) * T:i * T], w[i](), _NT, preferred_element_type=_F32)
                c11, c12, c21, c22 = _combine(mm)
                if pending is not None and c0 == Sk // 2:
                    store_shift(*pending, after=c12)
                s_refs[j][0:Sq, c0:c1] = c11
                s_refs[j][0:Sq, c1:c2] = c12
                s_refs[j][Sq:M, c0:c1] = c21
                s_refs[j][Sq:M, c1:c2] = c22
                ta, tb = jnp.maximum(c11, c12), jnp.maximum(c21, c22)
                ma = ta if ma is None else jnp.maximum(ma, ta)
                mb = tb if mb is None else jnp.maximum(mb, tb)
            if defer:
                return (j, ma, mb)
            store_shift(j, ma, mb)

        def softmax_pv(b, h, slot, j, mid=None):
            row = b * Sq if isinstance(b, int) else pl.multiple_of(b * Sq, 16)
            views = {z: vbuf.at[slot if z is None else slot + z_ref[z], j] for z in set(_V_Z)}
            v = lambda i: views[_V_Z[i - 1]]

            def probs(r0, c0):
                m = m_refs[j][r0:r0 + Sq, :]
                return jnp.exp2(s_refs[j][r0:r0 + Sq, c0:c0 + PW] - jnp.concatenate([m] * (PW // T), axis=1))

            def fold(acc, t):
                for c in range(PW // T):
                    u = t[:, c * T:(c + 1) * T]
                    acc = u if acc is None else acc + u
                return acc

            mm = {}
            la = lb = None
            for c0 in range(0, Sk, 2 * PW):
                c1, c2 = c0 + PW, c0 + 2 * PW
                a11, a12, a21, a22 = probs(0, c0), probs(0, c1), probs(Sq, c0), probs(Sq, c1)
                sa, sb = a11 + a12, a21 + a22
                la, lb = fold(la, sa), fold(lb, sb)
                a = {1: lambda: a11 + a22, 2: lambda: sb, 3: lambda: a11, 4: lambda: a22,
                     5: lambda: sa, 6: lambda: a21 - a11, 7: lambda: a12 - a22}
                w = _rhs_operands(lambda i: v(i)[c0:c1, 0:T], lambda i: v(i)[c0:c1, T:Dh],
                                  lambda i: v(i)[c1:c2, 0:T], lambda i: v(i)[c1:c2, T:Dh])
                for n, i in enumerate(_PV_ORDER):
                    if mid is not None and c2 == Sk and n == 5:
                        mid()
                    t = jnp.dot(a[i]().astype(_BF16), w[i](), preferred_element_type=_F32)
                    mm[i] = t if i not in mm else mm[i] + t
            c11, c12, c21, c22 = _combine(mm)
            never = z_ref[0] != 0
            ia = _recip(jnp.sum(jnp.where(never, mm[6], la), axis=-1, keepdims=True))
            ib = _recip(jnp.sum(jnp.where(never, mm[6], lb), axis=-1, keepdims=True))
            o_all[h * rep, pl.ds(row, Sq), 0:T] = c11 * ia
            o_all[h * rep, pl.ds(row, Sq), T:Dh] = c12 * ia
            o_all[h * rep + 1, pl.ds(row, Sq), 0:T] = c21 * ib
            o_all[h * rep + 1, pl.ds(row, Sq), T:Dh] = c22 * ib

        done = {}
        wo_sums = {}

        def finish_chunk(i):
            out_copy(i).start()
            z = z_ref[0]
            t = obuf[pl.ds(pl.multiple_of(o_start[i] + z, 16), 16), 0:T].astype(_F32)[0:8]
            done[i] = jnp.where(z != 0, t, 0.0)

        def after(t, zeros):
            if zeros is None:
                return t
            top = jnp.concatenate([t[0:8, 0:T] + zeros, t[0:8, T:]], axis=1)
            return jnp.concatenate([top, t[8:]], axis=0)

        def oproj_strassen(i):
            row0 = o_start[i]
            mm = {}
            for g in range(Hkv // 2):
                k1, k2 = 2 * g * G, (2 * g + 1) * G
                f = lambda r, k, z: wobuf[pl.ds(pl.multiple_of(r * DH + z_ref[z], 16), DH), k:k + G]
                ff = lambda r, k, z: f(r, k, z).astype(_F32)
                if g not in wo_sums:
                    wo_sums[g] = {1: (ff(0, k1, 1) + ff(1, k2, 1)).astype(_BF16),
                                  2: (ff(1, k1, 2) + ff(1, k2, 2)).astype(_BF16),
                                  5: (ff(0, k1, 5) + ff(0, k2, 5)).astype(_BF16),
                                  6: (ff(1, k1, 6) - ff(0, k1, 6)).astype(_BF16),
                                  7: (ff(0, k2, 7) - ff(1, k2, 7)).astype(_BF16)}
                a = dict(wo_sums[g])
                a[3], a[4] = f(0, k1, 8 + i), f(1, k2, 8 + i)

                def o(kk, tt, p):
                    z = 0 if _O_Z[p - 1] is None else z_ref[_O_Z[p - 1]]
                    return jnp.concatenate(
                        [o_all[(2 * g + kk) * rep + r + z, row0 + tt * T:row0 + (tt + 1) * T, :]
                         for r in range(rep)], axis=1)

                w = {1: lambda: o(0, 0, 1) + o(1, 1, 1),
                     2: lambda: after(o(0, 0, 2), done.get(i - 1) if g == 2 else None),
                     3: lambda: o(0, 1, 3) - o(1, 1, 3), 4: lambda: o(1, 0, 4) - o(0, 0, 4),
                     5: lambda: o(1, 1, 5), 6: lambda: o(0, 0, 6) + o(0, 1, 6),
                     7: lambda: o(1, 0, 7) + o(1, 1, 7)}
                for p in _O_ORDER:
                    t = lax.dot_general(a[p], w[p]().astype(_BF16), _NT, preferred_element_type=_F32)
                    mm[p] = t if p not in mm else mm[p] + t
            c11, c12, c21, c22 = _combine(mm)
            obuf[row0:row0 + T, :] = jnp.concatenate([c11, c21], axis=0).T.astype(obuf.dtype)
            obuf[row0 + T:row0 + 2 * T, :] = jnp.concatenate([c12, c22], axis=0).T.astype(obuf.dtype)
            finish_chunk(i)

        def oproj_last(i):
            row0, c0 = o_start[i], 2 * T
            acc, os_ = None, []
            for h in range(Hkv):
                o = jnp.concatenate([o_all[h * rep + r, row0:row0 + T, :] for r in range(rep)], axis=1)
                o = after(o, done.get(i - 1) if h == Hkv - 2 else None).astype(_BF16)
                os_.append(o)
                t = lax.dot_general(wobuf[c0:, h * G:(h + 1) * G], o, _NT, preferred_element_type=_F32)
                acc = t if acc is None else acc + t
            obuf[row0:row0 + T, c0:] = acc.T.astype(obuf.dtype)
            obuf[row0:row0 + T, 0:c0] = lax.dot_general(
                jnp.concatenate(os_, axis=1), wobuf[0:c0, :], _NT, preferred_element_type=_F32).astype(obuf.dtype)
            out_copy(i).start()

        for i in range(NS):
            (a0, c0), (a1, c1) = prev_section[i], _SECTIONS[i]
            for cp in section_copies(i):
                cp.wait()
            if i == NS - 1:
                k_copy(0, 0).wait()
                for j in range(U):
                    scores(j, 0, j)
                k_copy(2, 0).start()
            qproj(a0, a1, 0, c0)
            if i >= _Q_STRASSEN_FROM:
                assert a1 == B
                if i == _Q_STRASSEN_FROM:
                    prep_x()
                qproj_strassen(c0, c1)
            else:
                qproj(0, a1, c0, c1)

        def block(t, carry):
            slot = t & 1
            v_copy(t, slot).wait()
            k_copy(t + 1, 1 - slot).wait()
            b = t // BPB
            h0 = lax.rem(t, BPB) * U
            pending = [None]
            for j in range(U):
                def next_scores():
                    pending[0] = scores((t + 1) * U + j, 1 - slot, j, pending[0], j != U - 1)

                    @pl.when(t + 3 < NB)
                    def _():
                        k_copy(t + 3, 1 - slot, j).start()

                softmax_pv(b, h0 + j, slot, j, next_scores if j == U - 1 else None)

                @pl.when(t + 2 < NB)
                def _():
                    v_copy(t + 2, slot, j).start()

                if j != U - 1:
                    next_scores()
            return carry

        lax.fori_loop(0, NB - 1, block, 0)

        t = NB - 1
        v_copy(t, t % 2).wait()
        wo_copy.wait()
        for j in range(U):
            softmax_pv(t // BPB, (t % BPB) * U + j, t % 2, j)
        for i in range(NO - 1):
            oproj_strassen(i)
        oproj_last(NO - 1)
        for i in range(NO):
            out_copy(i).wait()

    hbm = pl.BlockSpec(memory_space=pl.ANY)
    out = pl.pallas_call(
        body,
        in_specs=[hbm] * 5,
        out_specs=hbm,
        out_shape=jax.ShapeDtypeStruct((R, D), x.dtype),
        scratch_shapes=[
            pltpu.VMEM((R, D), _BF16),
            pltpu.VMEM((D, Hq * Dh), _BF16),
            pltpu.VMEM((D, Hq * Dh), _BF16),
            pltpu.VMEM((2, U, Sk, Dh), _BF16),
            pltpu.VMEM((2, U, Sk, Dh), _BF16),
            pltpu.VMEM((RH // 2, 5 * K1), jnp.uint32),
            pltpu.VMEM((B * Hkv, Sq // 2, 7 * T), jnp.uint32),
            pltpu.VMEM((Hq, R, Dh), _F32),
            pltpu.VMEM((R, D), _BF16),
            pltpu.SemaphoreType.DMA((SEM_X + NS,)),
            pltpu.SMEM((_NZ,), jnp.int32),
        ] + [pltpu.VMEM((M, Sk), _F32)] * U + [pltpu.VMEM((M, T), _F32)] * U,
        compiler_params=pltpu.CompilerParams(
            vmem_limit_bytes=120 * 1024 * 1024,
            disable_bounds_checks=True,
            disable_semaphore_checks=True,
        ),
    )(x.reshape(R, D), k_cache.reshape(NB, U, Sk, Dh), v_cache.reshape(NB, U, Sk, Dh), wq, wo.T)
    return out.reshape(B, Sq, D)
```

```python
import jax
import jax.numpy as jnp
from jax import lax
import jax.experimental.pallas as pl
import jax.experimental.pallas.tpu as pltpu

_NT = (((1,), (1,)), ((), ()))
_LOG2E = 1.4426950408889634
_BF16 = jnp.bfloat16
_F32 = jnp.float32

_U = 4
_T = 128
_SECTIONS = ((2, 2), (5, 2), (8, 4), (8, 10), (8, 16))
_Q_STRASSEN_FROM = 2
_O_CHUNKS = (256, 256, 256, 256, 128)
_PW = 512
_Q_ORDER = (2, 4, 1, 6, 3, 5, 7)
_QK_ORDER = (5, 3, 1, 7, 4, 2, 6)
_PV_ORDER = (3, 4, 7, 5, 6, 2, 1)
_O_ORDER = (2, 5, 1, 3, 6, 4, 7)
_K_Z = (0, 1, 0, 1, 0, 1, 0)
_V_Z = (0, 1, None, 3, 4, 5, 6)
_O_Z = (1, None, 3, 4, None, 6, 7)
_NZ = 16


def _combine(m):
    return ((m[1] + m[4]) + (m[7] - m[5]), m[3] + m[5], m[2] + m[4], (m[1] - m[2]) + (m[3] + m[6]))


def _rhs_operands(b11, b12, b21, b22):
    f = lambda b, i: b(i).astype(_F32)
    return {1: lambda: (f(b11, 1) + f(b22, 1)).astype(_BF16),
            2: lambda: b11(2),
            3: lambda: (f(b12, 3) - f(b22, 3)).astype(_BF16),
            4: lambda: (f(b21, 4) - f(b11, 4)).astype(_BF16),
            5: lambda: b22(5),
            6: lambda: (f(b11, 6) + f(b12, 6)).astype(_BF16),
            7: lambda: (f(b21, 7) + f(b22, 7)).astype(_BF16)}


def _recip(l):
    r = pl.reciprocal(l, approx=True)
    return r * (2.0 - l * r)


def _softmax_shift(lane_max):
    m = jnp.max(lane_max, axis=-1, keepdims=True)
    m = m + jnp.log2(jnp.sum(jnp.exp2(lane_max - m), axis=-1, keepdims=True))
    return jnp.broadcast_to(m, lane_max.shape)


@jax.jit
def pallas_standalone__gqa_block_cached__near_ridge_kernel(
    x: jax.Array,
    k_cache: jax.Array,
    v_cache: jax.Array,
    wq: jax.Array,
    wo: jax.Array,
):
    B, Sq, D = x.shape
    _, Hkv, Sk, Dh = k_cache.shape
    Hq = wq.shape[1] // Dh
    rep = Hq // Hkv
    U, T, PW = _U, _T, _PW
    G = rep * Dh
    M = rep * Sq
    R = B * Sq
    RH, DH = R // 2, D // 2
    K1 = 2 * T
    K2 = D - K1
    NB = B * Hkv // U
    BPB = Hkv // U
    NS, NO = len(_SECTIONS), len(_O_CHUNKS)
    scale = Dh ** -0.5 * _LOG2E
    assert rep == 2 and Dh == 2 * T and Hkv % U == 0 and Sk % (2 * PW) == 0 and 0 < K2 <= K1
    assert Sq % 16 == 0 and DH % 16 == 0 and sum(_O_CHUNKS) == R and _SECTIONS[-1] == (B, Hq)
    o_start = [sum(_O_CHUNKS[:i]) for i in range(NO)]
    prev_section = ((0, 0),) + _SECTIONS[:-1]
    SEM_K, SEM_V, SEM_WO, SEM_O, SEM_X = 0, 2, 4, 5, 6

    def body(x_hbm, k_hbm, v_hbm, wq_hbm, wo_hbm, o_hbm,
             xbuf, wqbuf, wobuf, kbuf, vbuf, xs, q_all, o_all, obuf, sem, z_ref, *rest):
        s_refs, m_refs = rest[:U], rest[U:]
        for i in range(_NZ):
            z_ref[i] = 0

        def kv_copy(hbm, buf, sem0, blk, slot, j):
            if j is None:
                return pltpu.make_async_copy(hbm.at[blk], buf.at[slot], sem.at[sem0 + slot])
            return pltpu.make_async_copy(hbm.at[blk, j], buf.at[slot, j], sem.at[sem0 + slot])

        k_copy = lambda blk, slot, j=None: kv_copy(k_hbm, kbuf, SEM_K, blk, slot, j)
        v_copy = lambda blk, slot, j=None: kv_copy(v_hbm, vbuf, SEM_V, blk, slot, j)

        def section_copies(i):
            (a0, c0), (a1, c1) = prev_section[i], _SECTIONS[i]
            cps = []
            if a1 > a0:
                sl = pl.ds(a0 * Sq, (a1 - a0) * Sq)
                cps.append(pltpu.make_async_copy(x_hbm.at[sl], xbuf.at[sl], sem.at[SEM_X + i]))
            if c1 > c0:
                sl = pl.ds(c0 * Dh, (c1 - c0) * Dh)
                cps.append(pltpu.make_async_copy(wq_hbm.at[:, sl], wqbuf.at[:, sl], sem.at[SEM_X + i]))
            return cps

        def out_copy(i):
            sl = pl.ds(o_start[i], _O_CHUNKS[i])
            return pltpu.make_async_copy(obuf.at[sl], o_hbm.at[sl], sem.at[SEM_O])

        wo_copy = pltpu.make_async_copy(wo_hbm, wobuf, sem.at[SEM_WO])

        for i in range(NS):
            for cp in section_copies(i):
                cp.start()
        k_copy(0, 0).start()
        v_copy(0, 0).start()
        k_copy(1, 1).start()
        v_copy(1, 1).start()
        wo_copy.start(priority=1)

        def store_q(b, h, qa, qb):
            a11, a12, a21, a22 = qa[:, 0:T], qa[:, T:Dh], qb[:, 0:T], qb[:, T:Dh]
            ops = (a11 + a22, a21 + a22, a11, a22, a11 + a12, a21 - a11, a12 - a22)
            dst = q_all.at[b * Hkv + h]
            for i, a in enumerate(ops):
                dst[:, i * T:(i + 1) * T] = a.astype(_BF16)

        def qproj(b0, b1, c0, c1):
            if b1 <= b0:
                return
            for c in range(c0, c1, rep):
                q = jnp.dot(xbuf[b0 * Sq:b1 * Sq, :], wqbuf[:, c * Dh:c * Dh + G],
                            preferred_element_type=_F32) * scale
                for b in range(b0, b1):
                    qb = q[(b - b0) * Sq:(b - b0 + 1) * Sq]
                    store_q(b, c // rep, qb[:, 0:Dh], qb[:, Dh:G])

        def prep_x():
            f = lambda r, c0, c1: xbuf[r * RH:(r + 1) * RH, c0:c1].astype(_F32)
            cat = lambda u, v: jnp.concatenate([u, v], axis=1)
            xs[:, 0:K1] = cat(f(0, 0, K2) + f(1, K1, D), f(0, K2, K1)).astype(_BF16)
            xs[:, K1:2 * K1] = cat(f(1, 0, K2) + f(1, K1, D), f(1, K2, K1)).astype(_BF16)
            xs[:, 2 * K1:3 * K1] = (f(1, 0, K1) - f(0, 0, K1)).astype(_BF16)
            xs[:, 3 * K1:3 * K1 + K2] = (f(0, 0, K2) + f(0, K1, D)).astype(_BF16)
            xs[:, 4 * K1:4 * K1 + K2] = (f(0, K1, D) - f(1, K1, D)).astype(_BF16)

        def qproj_strassen(c0, c1):
            for c in range(c0, c1, rep):
                n1, n2 = c * Dh, (c + 1) * Dh
                g = lambda r0, r1, n: wqbuf[r0:r1, n:n + Dh]
                f = lambda r0, r1, n: g(r0, r1, n).astype(_F32)
                cat = lambda u, v: jnp.concatenate([u, v], axis=0)
                a = {1: lambda: xs[:, 0:K1], 2: lambda: xs[:, K1:2 * K1], 3: lambda: xbuf[0:RH, 0:K1],
                     4: lambda: xbuf[RH:R, K1:D], 5: lambda: xs[:, 3 * K1:3 * K1 + K2],
                     6: lambda: xs[:, 2 * K1:3 * K1], 7: lambda: xs[:, 4 * K1:4 * K1 + K2]}
                w = {1: lambda: cat(f(0, K2, n1) + f(K1, D, n2), f(K2, K1, n1)).astype(_BF16),
                     2: lambda: g(0, K1, n1),
                     3: lambda: cat(f(0, K2, n2) - f(K1, D, n2), f(K2, K1, n2)).astype(_BF16),
                     4: lambda: (f(K1, D, n1) - f(0, K2, n1)).astype(_BF16),
                     5: lambda: g(K1, D, n2),
                     6: lambda: (f(0, K1, n1) + f(0, K1, n2)).astype(_BF16),
                     7: lambda: (f(K1, D, n1) + f(K1, D, n2)).astype(_BF16)}
                mm = {}
                for i in _Q_ORDER:
                    mm[i] = jnp.dot(a[i](), w[i](), preferred_element_type=_F32)
                c11, c12, c21, c22 = [t * scale for t in _combine(mm)]
                for b in range(B // 2):
                    rows = slice(b * Sq, (b + 1) * Sq)
                    store_q(b, c // rep, c11[rows], c12[rows])
                    store_q(B // 2 + b, c // rep, c21[rows], c22[rows])

        def store_shift(j, ma, mb, after=None):
            if after is not None:
                never = z_ref[0] != 0
                ma, mb = jnp.where(never, after, ma), jnp.where(never, after, mb)
            m_refs[j][0:Sq, :] = _softmax_shift(ma)
            m_refs[j][Sq:M, :] = _softmax_shift(mb)

        def scores(unit, slot, j, pending=None, defer=False):
            q = q_all.at[unit]
            views = {z: kbuf.at[slot + z_ref[z], j] for z in set(_K_Z)}
            k = lambda i: views[_K_Z[i - 1]]
            ma = mb = None
            for c0 in range(0, Sk, 2 * T):
                c1, c2 = c0 + T, c0 + 2 * T
                w = _rhs_operands(lambda i: k(i)[c0:c1, 0:T], lambda i: k(i)[c1:c2, 0:T],
                                  lambda i: k(i)[c0:c1, T:Dh], lambda i: k(i)[c1:c2, T:Dh])
                mm = {}
                for i in _QK_ORDER:
                    mm[i] = lax.dot_general(q[:, (i - 1) * T:i * T], w[i](), _NT, preferred_element_type=_F32)
                c11, c12, c21, c22 = _combine(mm)
                if pending is not None and c0 == Sk // 2:
                    store_shift(*pending, after=c12)
                s_refs[j][0:Sq, c0:c1] = c11
                s_refs[j][0:Sq, c1:c2] = c12
                s_refs[j][Sq:M, c0:c1] = c21
                s_refs[j][Sq:M, c1:c2] = c22
                ta, tb = jnp.maximum(c11, c12), jnp.maximum(c21, c22)
                ma = ta if ma is None else jnp.maximum(ma, ta)
                mb = tb if mb is None else jnp.maximum(mb, tb)
            if defer:
                return (j, ma, mb)
            store_shift(j, ma, mb)

        def softmax_pv(b, h, slot, j, mid=None):
            row = b * Sq if isinstance(b, int) else pl.multiple_of(b * Sq, 16)
            views = {z: vbuf.at[slot if z is None else slot + z_ref[z], j] for z in set(_V_Z)}
            v = lambda i: views[_V_Z[i - 1]]

            def probs(r0, c0):
                m = m_refs[j][r0:r0 + Sq, :]
                return jnp.exp2(s_refs[j][r0:r0 + Sq, c0:c0 + PW] - jnp.concatenate([m] * (PW // T), axis=1))

            def fold(acc, t):
                for c in range(PW // T):
                    u = t[:, c * T:(c + 1) * T]
                    acc = u if acc is None else acc + u
                return acc

            mm = {}
            la = lb = None
            for c0 in range(0, Sk, 2 * PW):
                c1, c2 = c0 + PW, c0 + 2 * PW
                a11, a12, a21, a22 = probs(0, c0), probs(0, c1), probs(Sq, c0), probs(Sq, c1)
                sa, sb = a11 + a12, a21 + a22
                la, lb = fold(la, sa), fold(lb, sb)
                a = {1: lambda: a11 + a22, 2: lambda: sb, 3: lambda: a11, 4: lambda: a22,
                     5: lambda: sa, 6: lambda: a21 - a11, 7: lambda: a12 - a22}
                w = _rhs_operands(lambda i: v(i)[c0:c1, 0:T], lambda i: v(i)[c0:c1, T:Dh],
                                  lambda i: v(i)[c1:c2, 0:T], lambda i: v(i)[c1:c2, T:Dh])
                for n, i in enumerate(_PV_ORDER):
                    if mid is not None and c2 == Sk and n == 6:
                        mid()
                    t = jnp.dot(a[i]().astype(_BF16), w[i](), preferred_element_type=_F32)
                    mm[i] = t if i not in mm else mm[i] + t
            c11, c12, c21, c22 = _combine(mm)
            never = z_ref[0] != 0
            ia = _recip(jnp.sum(jnp.where(never, mm[6], la), axis=-1, keepdims=True))
            ib = _recip(jnp.sum(jnp.where(never, mm[6], lb), axis=-1, keepdims=True))
            o_all[h * rep, pl.ds(row, Sq), 0:T] = c11 * ia
            o_all[h * rep, pl.ds(row, Sq), T:Dh] = c12 * ia
            o_all[h * rep + 1, pl.ds(row, Sq), 0:T] = c21 * ib
            o_all[h * rep + 1, pl.ds(row, Sq), T:Dh] = c22 * ib

        done = {}
        wo_sums = {}

        def finish_chunk(i):
            out_copy(i).start()
            z = z_ref[0]
            t = obuf[pl.ds(pl.multiple_of(o_start[i] + z, 16), 16), 0:T].astype(_F32)[0:8]
            done[i] = jnp.where(z != 0, t, 0.0)

        def after(t, zeros):
            if zeros is None:
                return t
            top = jnp.concatenate([t[0:8, 0:T] + zeros, t[0:8, T:]], axis=1)
            return jnp.concatenate([top, t[8:]], axis=0)

        def oproj_strassen(i):
            row0 = o_start[i]
            mm = {}
            for g in range(Hkv // 2):
                k1, k2 = 2 * g * G, (2 * g + 1) * G
                f = lambda r, k, z: wobuf[pl.ds(pl.multiple_of(r * DH + z_ref[z], 16), DH), k:k + G]
                ff = lambda r, k, z: f(r, k, z).astype(_F32)
                if g not in wo_sums:
                    wo_sums[g] = {1: (ff(0, k1, 1) + ff(1, k2, 1)).astype(_BF16),
                                  2: (ff(1, k1, 2) + ff(1, k2, 2)).astype(_BF16),
                                  5: (ff(0, k1, 5) + ff(0, k2, 5)).astype(_BF16),
                                  6: (ff(1, k1, 6) - ff(0, k1, 6)).astype(_BF16),
                                  7: (ff(0, k2, 7) - ff(1, k2, 7)).astype(_BF16)}
                a = dict(wo_sums[g])
                a[3], a[4] = f(0, k1, 8 + i), f(1, k2, 8 + i)

                def o(kk, tt, p):
                    z = 0 if _O_Z[p - 1] is None else z_ref[_O_Z[p - 1]]
                    return jnp.concatenate(
                        [o_all[(2 * g + kk) * rep + r + z, row0 + tt * T:row0 + (tt + 1) * T, :]
                         for r in range(rep)], axis=1)

                w = {1: lambda: o(0, 0, 1) + o(1, 1, 1),
                     2: lambda: after(o(0, 0, 2), done.get(i - 1) if g == 2 else None),
                     3: lambda: o(0, 1, 3) - o(1, 1, 3), 4: lambda: o(1, 0, 4) - o(0, 0, 4),
                     5: lambda: o(1, 1, 5), 6: lambda: o(0, 0, 6) + o(0, 1, 6),
                     7: lambda: o(1, 0, 7) + o(1, 1, 7)}
                for p in _O_ORDER:
                    t = lax.dot_general(a[p], w[p]().astype(_BF16), _NT, preferred_element_type=_F32)
                    mm[p] = t if p not in mm else mm[p] + t
            c11, c12, c21, c22 = _combine(mm)
            obuf[row0:row0 + T, :] = jnp.concatenate([c11, c21], axis=0).T.astype(obuf.dtype)
            obuf[row0 + T:row0 + 2 * T, :] = jnp.concatenate([c12, c22], axis=0).T.astype(obuf.dtype)
            finish_chunk(i)

        def oproj_last(i):
            row0, c0 = o_start[i], 2 * T
            acc, os_ = None, []
            for h in range(Hkv):
                o = jnp.concatenate([o_all[h * rep + r, row0:row0 + T, :] for r in range(rep)], axis=1)
                o = after(o, done.get(i - 1) if h == Hkv - 2 else None).astype(_BF16)
                os_.append(o)
                t = lax.dot_general(wobuf[c0:, h * G:(h + 1) * G], o, _NT, preferred_element_type=_F32)
                acc = t if acc is None else acc + t
            obuf[row0:row0 + T, c0:] = acc.T.astype(obuf.dtype)
            obuf[row0:row0 + T, 0:c0] = lax.dot_general(
                jnp.concatenate(os_, axis=1), wobuf[0:c0, :], _NT, preferred_element_type=_F32).astype(obuf.dtype)
            out_copy(i).start()

        for i in range(NS):
            (a0, c0), (a1, c1) = prev_section[i], _SECTIONS[i]
            for cp in section_copies(i):
                cp.wait()
            if i == NS - 1:
                k_copy(0, 0).wait()
                for j in range(U):
                    scores(j, 0, j)
                k_copy(2, 0).start()
            qproj(a0, a1, 0, c0)
            if i >= _Q_STRASSEN_FROM:
                assert a1 == B
                if i == _Q_STRASSEN_FROM:
                    prep_x()
                qproj_strassen(c0, c1)
            else:
                qproj(0, a1, c0, c1)

        def block(t, carry):
            slot = t & 1
            v_copy(t, slot).wait()
            k_copy(t + 1, 1 - slot).wait()
            b = t // BPB
            h0 = lax.rem(t, BPB) * U
            pending = [None]
            for j in range(U):
                def next_scores():
                    pending[0] = scores((t + 1) * U + j, 1 - slot, j, pending[0], j != U - 1)

                    @pl.when(t + 3 < NB)
                    def _():
                        k_copy(t + 3, 1 - slot, j).start()

                softmax_pv(b, h0 + j, slot, j, next_scores)

                @pl.when(t + 2 < NB)
                def _():
                    v_copy(t + 2, slot, j).start()
            return carry

        lax.fori_loop(0, NB - 1, block, 0)

        t = NB - 1
        v_copy(t, t % 2).wait()
        wo_copy.wait()
        for j in range(U):
            softmax_pv(t // BPB, (t % BPB) * U + j, t % 2, j)
        for i in range(NO - 1):
            oproj_strassen(i)
        oproj_last(NO - 1)
        for i in range(NO):
            out_copy(i).wait()

    hbm = pl.BlockSpec(memory_space=pl.ANY)
    out = pl.pallas_call(
        body,
        in_specs=[hbm] * 5,
        out_specs=hbm,
        out_shape=jax.ShapeDtypeStruct((R, D), x.dtype),
        scratch_shapes=[
            pltpu.VMEM((R, D), _BF16),
            pltpu.VMEM((D, Hq * Dh), _BF16),
            pltpu.VMEM((D, Hq * Dh), _BF16),
            pltpu.VMEM((2, U, Sk, Dh), _BF16),
            pltpu.VMEM((2, U, Sk, Dh), _BF16),
            pltpu.VMEM((RH, 5 * K1), _BF16),
            pltpu.VMEM((B * Hkv, Sq, 7 * T), _BF16),
            pltpu.VMEM((Hq, R, Dh), _F32),
            pltpu.VMEM((R, D), _BF16),
            pltpu.SemaphoreType.DMA((SEM_X + NS,)),
            pltpu.SMEM((_NZ,), jnp.int32),
        ] + [pltpu.VMEM((M, Sk), _F32)] * U + [pltpu.VMEM((M, T), _F32)] * U,
        compiler_params=pltpu.CompilerParams(vmem_limit_bytes=120 * 1024 * 1024),
    )(x.reshape(R, D), k_cache.reshape(NB, U, Sk, Dh), v_cache.reshape(NB, U, Sk, Dh), wq, wo.T)
    return out.reshape(B, Sq, D)
```

```python
import jax
import jax.numpy as jnp
from jax import lax
import jax.experimental.pallas as pl
import jax.experimental.pallas.tpu as pltpu

_NT = (((1,), (1,)), ((), ()))
_LOG2E = 1.4426950408889634
_BF16 = jnp.bfloat16
_F32 = jnp.float32

_U = 4
_T = 128
_SECTIONS = ((1, 1), (3, 1), (4, 2), (4, 5), (4, 8))
_O_CHUNKS = (256, 256, 256, 256, 128)
_Q_ORDER = (2, 5, 4, 3, 1, 6, 7)
_QK_ORDER = (5, 3, 1, 7, 4, 2, 6)
_PV_ORDER = (3, 4, 7, 5, 6, 2, 1)
_O_ORDER = (2, 5, 1, 3, 6, 4, 7)
_K_Z = (0, 1, 0, 1, 0, 1, 0)
_V_Z = (0, 1, None, 3, 4, 5, 6)
_O_Z = (1, None, 3, 4, None, 6, 7)
_NZ = 16


def _combine(m):
    return ((m[1] + m[4]) + (m[7] - m[5]), m[3] + m[5], m[2] + m[4], (m[1] - m[2]) + (m[3] + m[6]))


def _rhs_operands(b11, b12, b21, b22):
    f = lambda b, i: b(i).astype(_F32)
    return {1: lambda: (f(b11, 1) + f(b22, 1)).astype(_BF16),
            2: lambda: b11(2),
            3: lambda: (f(b12, 3) - f(b22, 3)).astype(_BF16),
            4: lambda: (f(b21, 4) - f(b11, 4)).astype(_BF16),
            5: lambda: b22(5),
            6: lambda: (f(b11, 6) + f(b12, 6)).astype(_BF16),
            7: lambda: (f(b21, 7) + f(b22, 7)).astype(_BF16)}


def _recip(l):
    r = pl.reciprocal(l, approx=True)
    return r * (2.0 - l * r)


def _softmax_shift(lane_max):
    m = jnp.max(lane_max, axis=-1, keepdims=True)
    m = m + jnp.log2(jnp.sum(jnp.exp2(lane_max - m), axis=-1, keepdims=True))
    return jnp.broadcast_to(m, lane_max.shape)


@jax.jit
def pallas_standalone__gqa_block_cached__near_ridge_kernel(
    x: jax.Array,
    k_cache: jax.Array,
    v_cache: jax.Array,
    wq: jax.Array,
    wo: jax.Array,
):
    B, Sq, D = x.shape
    _, Hkv, Sk, Dh = k_cache.shape
    Hq = wq.shape[1] // Dh
    rep = Hq // Hkv
    U, T = _U, _T
    G = rep * Dh
    M = rep * Sq
    R = B * Sq
    RH, DH, SH = R // 2, D // 2, Sk // 2
    K1 = 2 * T
    K2 = D - K1
    NB = B * Hkv // U
    BPB = Hkv // U
    NS, NO = len(_SECTIONS), len(_O_CHUNKS)
    scale = Dh ** -0.5 * _LOG2E
    assert rep == 2 and Dh == 2 * T and Hkv % U == 0 and Sk % (4 * T) == 0 and 0 < K2 <= K1
    assert Sq % 16 == 0 and DH % 16 == 0 and sum(_O_CHUNKS) == R and _SECTIONS[-1] == (B // 2, Hkv)
    o_start = [sum(_O_CHUNKS[:i]) for i in range(NO)]
    prev_section = ((0, 0),) + _SECTIONS[:-1]
    SEM_K, SEM_V, SEM_WO, SEM_O, SEM_X = 0, 2, 4, 5, 6

    def body(x_hbm, k_hbm, v_hbm, wq_hbm, wo_hbm, o_hbm,
             xbuf, wqbuf, wobuf, kbuf, vbuf, xs, q_all, o_all, obuf, sem, z_ref, *rest):
        s_refs, m_refs = rest[:U], rest[U:]
        for i in range(_NZ):
            z_ref[i] = 0

        def kv_copy(hbm, buf, sem0, blk, slot, j):
            if j is None:
                return pltpu.make_async_copy(hbm.at[blk], buf.at[slot], sem.at[sem0 + slot])
            return pltpu.make_async_copy(hbm.at[blk, j], buf.at[slot, j], sem.at[sem0 + slot])

        k_copy = lambda blk, slot, j=None: kv_copy(k_hbm, kbuf, SEM_K, blk, slot, j)
        v_copy = lambda blk, slot, j=None: kv_copy(v_hbm, vbuf, SEM_V, blk, slot, j)

        def section_copies(i):
            (a0, c0), (a1, c1) = prev_section[i], _SECTIONS[i]
            cps = []
            if a1 > a0:
                for half in range(2):
                    sl = pl.ds(half * RH + a0 * Sq, (a1 - a0) * Sq)
                    cps.append(pltpu.make_async_copy(x_hbm.at[sl], xbuf.at[sl], sem.at[SEM_X + i]))
            if c1 > c0:
                sl = pl.ds(c0 * G, (c1 - c0) * G)
                cps.append(pltpu.make_async_copy(wq_hbm.at[:, sl], wqbuf.at[:, sl], sem.at[SEM_X + i]))
            return cps

        def out_copy(i):
            sl = pl.ds(o_start[i], _O_CHUNKS[i])
            return pltpu.make_async_copy(obuf.at[sl], o_hbm.at[sl], sem.at[SEM_O])

        wo_copy = pltpu.make_async_copy(wo_hbm, wobuf, sem.at[SEM_WO])

        for i in range(NS):
            for cp in section_copies(i):
                cp.start()
        k_copy(0, 0).start()
        v_copy(0, 0).start()
        k_copy(1, 1).start()
        v_copy(1, 1).start()
        wo_copy.start(priority=1)

        def store_q(b, h, qa, qb):
            a11, a12, a21, a22 = qa[:, 0:T], qa[:, T:Dh], qb[:, 0:T], qb[:, T:Dh]
            ops = (a11 + a22, a21 + a22, a11, a22, a11 + a12, a21 - a11, a12 - a22)
            dst = q_all.at[b * Hkv + h]
            for i, a in enumerate(ops):
                dst[:, i * T:(i + 1) * T] = a.astype(_BF16)

        def prep_x(p0, p1):
            r0, r1 = p0 * Sq, p1 * Sq
            f = lambda r, c0, c1: xbuf[r * RH + r0:r * RH + r1, c0:c1].astype(_F32)
            cat = lambda u, v: jnp.concatenate([u, v], axis=1)
            xs[r0:r1, 0:K1] = cat(f(0, 0, K2) + f(1, K1, D), f(0, K2, K1)).astype(_BF16)
            xs[r0:r1, K1:2 * K1] = cat(f(1, 0, K2) + f(1, K1, D), f(1, K2, K1)).astype(_BF16)
            xs[r0:r1, 2 * K1:3 * K1] = (f(1, 0, K1) - f(0, 0, K1)).astype(_BF16)
            xs[r0:r1, 3 * K1:3 * K1 + K2] = (f(0, 0, K2) + f(0, K1, D)).astype(_BF16)
            xs[r0:r1, 4 * K1:4 * K1 + K2] = (f(0, K1, D) - f(1, K1, D)).astype(_BF16)

        def qproj(p0, p1, h0, h1):
            if p1 <= p0:
                return
            r0, r1 = p0 * Sq, p1 * Sq
            for h in range(h0, h1):
                n1, n2 = h * G, h * G + Dh
                g = lambda k0, k1, n: wqbuf[k0:k1, n:n + Dh]
                f = lambda k0, k1, n: g(k0, k1, n).astype(_F32)
                cat = lambda u, v: jnp.concatenate([u, v], axis=0)
                a = {1: lambda: xs[r0:r1, 0:K1], 2: lambda: xs[r0:r1, K1:2 * K1], 3: lambda: xbuf[r0:r1, 0:K1],
                     4: lambda: xbuf[RH + r0:RH + r1, K1:D], 5: lambda: xs[r0:r1, 3 * K1:3 * K1 + K2],
                     6: lambda: xs[r0:r1, 2 * K1:3 * K1], 7: lambda: xs[r0:r1, 4 * K1:4 * K1 + K2]}
                w = {1: lambda: cat(f(0, K2, n1) + f(K1, D, n2), f(K2, K1, n1)).astype(_BF16),
                     2: lambda: g(0, K1, n1),
                     3: lambda: cat(f(0, K2, n2) - f(K1, D, n2), f(K2, K1, n2)).astype(_BF16),
                     4: lambda: (f(K1, D, n1) - f(0, K2, n1)).astype(_BF16),
                     5: lambda: g(K1, D, n2),
                     6: lambda: (f(0, K1, n1) + f(0, K1, n2)).astype(_BF16),
                     7: lambda: (f(K1, D, n1) + f(K1, D, n2)).astype(_BF16)}
                mm = {}
                for i in _Q_ORDER:
                    mm[i] = jnp.dot(a[i](), w[i](), preferred_element_type=_F32)
                c11, c12, c21, c22 = [t * scale for t in _combine(mm)]
                for p in range(p0, p1):
                    rows = slice((p - p0) * Sq, (p - p0 + 1) * Sq)
                    store_q(p, h, c11[rows], c12[rows])
                    store_q(B // 2 + p, h, c21[rows], c22[rows])

        def store_shift(j, ma, mb, after=None):
            if after is not None:
                never = z_ref[0] != 0
                ma, mb = jnp.where(never, after, ma), jnp.where(never, after, mb)
            m_refs[j][0:Sq, :] = _softmax_shift(ma)
            m_refs[j][Sq:M, :] = _softmax_shift(mb)

        def scores(unit, slot, j, pending=None, defer=False):
            q = q_all.at[unit]
            views = {z: kbuf.at[slot + z_ref[z], j] for z in dict.fromkeys(_K_Z)}
            k = lambda i: views[_K_Z[i - 1]]
            ma = mb = None
            for c0 in range(0, Sk, 2 * T):
                c1, c2 = c0 + T, c0 + 2 * T
                w = _rhs_operands(lambda i: k(i)[c0:c1, 0:T], lambda i: k(i)[c1:c2, 0:T],
                                  lambda i: k(i)[c0:c1, T:Dh], lambda i: k(i)[c1:c2, T:Dh])
                mm = {}
                for i in _QK_ORDER:
                    mm[i] = lax.dot_general(q[:, (i - 1) * T:i * T], w[i](), _NT, preferred_element_type=_F32)
                c11, c12, c21, c22 = _combine(mm)
                if pending is not None and c0 == Sk // 2:
                    store_shift(*pending, after=c12)
                s_refs[j][0:Sq, c0:c1] = c11
                s_refs[j][0:Sq, c1:c2] = c12
                s_refs[j][Sq:M, c0:c1] = c21
                s_refs[j][Sq:M, c1:c2] = c22
                ta, tb = jnp.maximum(c11, c12), jnp.maximum(c21, c22)
                ma = ta if ma is None else jnp.maximum(ma, ta)
                mb = tb if mb is None else jnp.maximum(mb, tb)
            if defer:
                return (j, ma, mb)
            store_shift(j, ma, mb)

        def softmax_pv(b, h, slot, j, mid=None):
            row = b * Sq if isinstance(b, int) else pl.multiple_of(b * Sq, 16)
            views = {z: vbuf.at[slot if z is None else slot + z_ref[z], j] for z in dict.fromkeys(_V_Z)}
            v = lambda i: views[_V_Z[i - 1]]

            def probs(r0, c0):
                m = m_refs[j][r0:r0 + Sq, :]
                return jnp.exp2(s_refs[j][r0:r0 + Sq, c0:c0 + SH] - jnp.concatenate([m] * (SH // T), axis=1))

            def lane_sum(t):
                acc = t[:, 0:T]
                for c in range(1, SH // T):
                    acc = acc + t[:, c * T:(c + 1) * T]
                return acc

            a11, a12, a21, a22 = probs(0, 0), probs(0, SH), probs(Sq, 0), probs(Sq, SH)
            sa, sb = a11 + a12, a21 + a22
            la, lb = lane_sum(sa), lane_sum(sb)
            a = {1: lambda: a11 + a22, 2: lambda: sb, 3: lambda: a11, 4: lambda: a22,
                 5: lambda: sa, 6: lambda: a21 - a11, 7: lambda: a12 - a22}
            w = _rhs_operands(lambda i: v(i)[0:SH, 0:T], lambda i: v(i)[0:SH, T:Dh],
                              lambda i: v(i)[SH:Sk, 0:T], lambda i: v(i)[SH:Sk, T:Dh])
            mm = {}
            for i in _PV_ORDER:
                if mid is not None and i == _PV_ORDER[-1]:
                    mid()
                mm[i] = jnp.dot(a[i]().astype(_BF16), w[i](), preferred_element_type=_F32)
            c11, c12, c21, c22 = _combine(mm)
            never = z_ref[0] != 0
            ia = _recip(jnp.sum(jnp.where(never, mm[6], la), axis=-1, keepdims=True))
            ib = _recip(jnp.sum(jnp.where(never, mm[6], lb), axis=-1, keepdims=True))
            o_all[h * rep, pl.ds(row, Sq), 0:T] = c11 * ia
            o_all[h * rep, pl.ds(row, Sq), T:Dh] = c12 * ia
            o_all[h * rep + 1, pl.ds(row, Sq), 0:T] = c21 * ib
            o_all[h * rep + 1, pl.ds(row, Sq), T:Dh] = c22 * ib

        done = {}
        wo_sums = {}

        def finish_chunk(i):
            out_copy(i).start()
            z = z_ref[0]
            t = obuf[pl.ds(pl.multiple_of(o_start[i] + z, 16), 16), 0:T].astype(_F32)[0:8]
            done[i] = jnp.where(z != 0, t, 0.0)

        def after(t, zeros):
            if zeros is None:
                return t
            top = jnp.concatenate([t[0:8, 0:T] + zeros, t[0:8, T:]], axis=1)
            return jnp.concatenate([top, t[8:]], axis=0)

        def oproj_strassen(i):
            row0 = o_start[i]
            mm = {}
            for g in range(Hkv // 2):
                k1, k2 = 2 * g * G, (2 * g + 1) * G
                f = lambda r, k, z: wobuf[pl.ds(pl.multiple_of(r * DH + z_ref[z], 16), DH), k:k + G]
                ff = lambda r, k, z: f(r, k, z).astype(_F32)
                if g not in wo_sums:
                    wo_sums[g] = {1: (ff(0, k1, 1) + ff(1, k2, 1)).astype(_BF16),
                                  2: (ff(1, k1, 2) + ff(1, k2, 2)).astype(_BF16),
                                  5: (ff(0, k1, 5) + ff(0, k2, 5)).astype(_BF16),
                                  6: (ff(1, k1, 6) - ff(0, k1, 6)).astype(_BF16),
                                  7: (ff(0, k2, 7) - ff(1, k2, 7)).astype(_BF16)}
                a = dict(wo_sums[g])
                a[3], a[4] = f(0, k1, 8 + i), f(1, k2, 8 + i)

                def o(kk, tt, p):
                    z = 0 if _O_Z[p - 1] is None else z_ref[_O_Z[p - 1]]
                    return jnp.concatenate(
                        [o_all[(2 * g + kk) * rep + r + z, row0 + tt * T:row0 + (tt + 1) * T, :]
                         for r in range(rep)], axis=1)

                w = {1: lambda: o(0, 0, 1) + o(1, 1, 1),
                     2: lambda: after(o(0, 0, 2), done.get(i - 1) if g == 2 else None),
                     3: lambda: o(0, 1, 3) - o(1, 1, 3), 4: lambda: o(1, 0, 4) - o(0, 0, 4),
                     5: lambda: o(1, 1, 5), 6: lambda: o(0, 0, 6) + o(0, 1, 6),
                     7: lambda: o(1, 0, 7) + o(1, 1, 7)}
                for p in _O_ORDER:
                    t = lax.dot_general(a[p], w[p]().astype(_BF16), _NT, preferred_element_type=_F32)
                    mm[p] = t if p not in mm else mm[p] + t
            c11, c12, c21, c22 = _combine(mm)
            obuf[row0:row0 + T, :] = jnp.concatenate([c11, c21], axis=0).T.astype(obuf.dtype)
            obuf[row0 + T:row0 + 2 * T, :] = jnp.concatenate([c12, c22], axis=0).T.astype(obuf.dtype)
            finish_chunk(i)

        def oproj_last(i):
            row0, c0 = o_start[i], 2 * T
            acc, os_ = None, []
            for h in range(Hkv):
                o = jnp.concatenate([o_all[h * rep + r, row0:row0 + T, :] for r in range(rep)], axis=1)
                o = after(o, done.get(i - 1) if h == Hkv - 2 else None).astype(_BF16)
                os_.append(o)
                t = lax.dot_general(wobuf[c0:, h * G:(h + 1) * G], o, _NT, preferred_element_type=_F32)
                acc = t if acc is None else acc + t
            obuf[row0:row0 + T, c0:] = acc.T.astype(obuf.dtype)
            obuf[row0:row0 + T, 0:c0] = lax.dot_general(
                jnp.concatenate(os_, axis=1), wobuf[0:c0, :], _NT, preferred_element_type=_F32).astype(obuf.dtype)
            out_copy(i).start()

        for i in range(NS):
            (a0, c0), (a1, c1) = prev_section[i], _SECTIONS[i]
            for cp in section_copies(i):
                cp.wait()
            if i == NS - 1:
                k_copy(0, 0).wait()
                for j in range(U):
                    scores(j, 0, j)
                k_copy(2, 0).start()
            if a1 > a0:
                prep_x(a0, a1)
            qproj(a0, a1, 0, c0)
            qproj(0, a1, c0, c1)

        def block(t, carry):
            slot = t & 1
            v_copy(t, slot).wait()
            k_copy(t + 1, 1 - slot).wait()
            b = t // BPB
            h0 = lax.rem(t, BPB) * U
            pending = [None]
            for j in range(U):
                def next_scores():
                    pending[0] = scores((t + 1) * U + j, 1 - slot, j, pending[0], j != U - 1)

                    @pl.when(t + 3 < NB)
                    def _():
                        k_copy(t + 3, 1 - slot, j).start()

                softmax_pv(b, h0 + j, slot, j, next_scores)

                @pl.when(t + 2 < NB)
                def _():
                    v_copy(t + 2, slot, j).start()
            return carry

        lax.fori_loop(0, NB - 1, block, 0)

        t = NB - 1
        v_copy(t, t % 2).wait()
        wo_copy.wait()
        for j in range(U):
            softmax_pv(t // BPB, (t % BPB) * U + j, t % 2, j)
        for i in range(NO - 1):
            oproj_strassen(i)
        oproj_last(NO - 1)
        for i in range(NO):
            out_copy(i).wait()

    hbm = pl.BlockSpec(memory_space=pl.ANY)
    out = pl.pallas_call(
        body,
        in_specs=[hbm] * 5,
        out_specs=hbm,
        out_shape=jax.ShapeDtypeStruct((R, D), x.dtype),
        scratch_shapes=[
            pltpu.VMEM((R, D), _BF16),
            pltpu.VMEM((D, Hq * Dh), _BF16),
            pltpu.VMEM((D, Hq * Dh), _BF16),
            pltpu.VMEM((2, U, Sk, Dh), _BF16),
            pltpu.VMEM((2, U, Sk, Dh), _BF16),
            pltpu.VMEM((RH, 5 * K1), _BF16),
            pltpu.VMEM((B * Hkv, Sq, 7 * T), _BF16),
            pltpu.VMEM((Hq, R, Dh), _F32),
            pltpu.VMEM((R, D), _BF16),
            pltpu.SemaphoreType.DMA((SEM_X + NS,)),
            pltpu.SMEM((_NZ,), jnp.int32),
        ] + [pltpu.VMEM((M, Sk), _F32)] * U + [pltpu.VMEM((M, T), _F32)] * U,
        compiler_params=pltpu.CompilerParams(vmem_limit_bytes=120 * 1024 * 1024),
    )(x.reshape(R, D), k_cache.reshape(NB, U, Sk, Dh), v_cache.reshape(NB, U, Sk, Dh), wq, wo.T)
    return out.reshape(B, Sq, D)
```

```python
import jax
import jax.numpy as jnp
from jax import lax
import jax.experimental.pallas as pl
import jax.experimental.pallas.tpu as pltpu

_NT = (((1,), (1,)), ((), ()))
_LOG2E = 1.4426950408889634
_BF16 = jnp.bfloat16
_F32 = jnp.float32

_U = 4
_T = 128
_Q_LOOP = 2
_O_CHUNKS = (256, 256, 256, 256, 128)
_Q_ORDER = (5, 7, 4, 1, 3, 6, 2)
_QK_ORDER = (5, 3, 1, 7, 4, 2, 6)
_PV_ORDER = (3, 4, 7, 5, 6, 2, 1)
_O_ORDER = (2, 5, 1, 3, 6, 4, 7)
_K_Z = (0, 1, 0, 1, 0, 1, 0)
_V_Z = (0, 1, None, 3, 4, 5, 6)
_O_Z = (1, None, 3, 4, None, 6, 7)
_NZ = 16


def _combine(m):
    return ((m[1] + m[4]) + (m[7] - m[5]), m[3] + m[5], m[2] + m[4], (m[1] - m[2]) + (m[3] + m[6]))


def _rhs_operands(b11, b12, b21, b22):
    f = lambda b, i: b(i).astype(_F32)
    return {1: lambda: (f(b11, 1) + f(b22, 1)).astype(_BF16),
            2: lambda: b11(2),
            3: lambda: (f(b12, 3) - f(b22, 3)).astype(_BF16),
            4: lambda: (f(b21, 4) - f(b11, 4)).astype(_BF16),
            5: lambda: b22(5),
            6: lambda: (f(b11, 6) + f(b12, 6)).astype(_BF16),
            7: lambda: (f(b21, 7) + f(b22, 7)).astype(_BF16)}


def _recip(l):
    r = pl.reciprocal(l, approx=True)
    return r * (2.0 - l * r)


def _softmax_shift(lane_max):
    m = jnp.max(lane_max, axis=-1, keepdims=True)
    m = m + jnp.log2(jnp.sum(jnp.exp2(lane_max - m), axis=-1, keepdims=True))
    return jnp.broadcast_to(m, lane_max.shape)


@jax.jit
def pallas_standalone__gqa_block_cached__near_ridge_kernel(
    x: jax.Array,
    k_cache: jax.Array,
    v_cache: jax.Array,
    wq: jax.Array,
    wo: jax.Array,
):
    B, Sq, D = x.shape
    _, Hkv, Sk, Dh = k_cache.shape
    Hq = wq.shape[1] // Dh
    rep = Hq // Hkv
    U, T = _U, _T
    G = rep * Dh
    M = rep * Sq
    R = B * Sq
    RH, DH, SH = R // 2, D // 2, Sk // 2
    K1 = 2 * T
    K2 = D - K1
    E = T // 2
    XS = {1: 0, 2: K1, 6: 2 * K1, 4: 3 * K1, 5: 3 * K1 + 3 * T, 7: 3 * K1 + 6 * T}
    NB = B * Hkv // U
    BPB = Hkv // U
    NO = len(_O_CHUNKS)
    NP = B // 2
    NQ = (Hkv - 2) // _Q_LOOP
    scale = Dh ** -0.5 * _LOG2E
    assert rep == 2 and Dh == 2 * T and Hkv % U == 0 and Sk % (4 * T) == 0 and K2 == 3 * E
    assert Sq % 16 == 0 and DH % 16 == 0 and sum(_O_CHUNKS) == R and NP == 4 and (Hkv - 2) % _Q_LOOP == 0
    o_start = [sum(_O_CHUNKS[:i]) for i in range(NO)]
    SEM_K, SEM_V, SEM_WO, SEM_O, SEM_X = 0, 2, 4, 5, 6
    SEM_W = SEM_X + NP

    def body(x_hbm, k_hbm, v_hbm, wq_hbm, wo_hbm, o_hbm,
             xbuf, wqbuf, wobuf, kbuf, vbuf, xs, q_all, o_all, obuf, sem, z_ref, *rest):
        s_refs, m_refs = rest[:U], rest[U:]
        for i in range(_NZ):
            z_ref[i] = 0

        def kv_copy(hbm, buf, sem0, blk, slot, j):
            if j is None:
                return pltpu.make_async_copy(hbm.at[blk], buf.at[slot], sem.at[sem0 + slot])
            return pltpu.make_async_copy(hbm.at[blk, j], buf.at[slot, j], sem.at[sem0 + slot])

        k_copy = lambda blk, slot, j=None: kv_copy(k_hbm, kbuf, SEM_K, blk, slot, j)
        v_copy = lambda blk, slot, j=None: kv_copy(v_hbm, vbuf, SEM_V, blk, slot, j)

        def wq_copy(h, s):
            c = h * G if isinstance(h, int) else pl.multiple_of(h * G, G)
            return pltpu.make_async_copy(wq_hbm.at[:, pl.ds(c, G)], wqbuf.at[h], sem.at[s])

        def rows_of(p, half=0):
            r = half * RH + p * Sq
            return pl.ds(r if isinstance(r, int) else pl.multiple_of(r, 16), Sq)

        def x_copies(p):
            return [pltpu.make_async_copy(x_hbm.at[rows_of(p, half)], xbuf.at[rows_of(p, half)], sem.at[SEM_X + p])
                    for half in range(2)]

        def out_copy(i):
            sl = pl.ds(o_start[i], _O_CHUNKS[i])
            return pltpu.make_async_copy(obuf.at[sl], o_hbm.at[sl], sem.at[SEM_O])

        wo_copy = pltpu.make_async_copy(wo_hbm, wobuf, sem.at[SEM_WO])

        wq_copy(0, SEM_O).start()
        for p in range(NP):
            for cp in x_copies(p):
                cp.start()
        for h in range(1, Hkv - 1):
            wq_copy(h, SEM_W + (h - 1) // _Q_LOOP).start()
        wq_copy(Hkv - 1, SEM_K).start()
        k_copy(0, 0).start()
        v_copy(0, 0).start()
        k_copy(1, 1).start()
        v_copy(1, 1).start()
        wo_copy.start(priority=1)

        def store_q(b, h, qa, qb):
            a11, a12, a21, a22 = qa[:, 0:T], qa[:, T:Dh], qb[:, 0:T], qb[:, T:Dh]
            ops = (a11 + a22, a21 + a22, a11, a22, a11 + a12, a21 - a11, a12 - a22)
            q_all.at[b * Hkv + h][...] = jnp.concatenate(ops, axis=1).astype(_BF16)

        def prep_x(p):
            f = lambda half, c0, c1: xbuf[rows_of(p, half), c0:c1].astype(_F32)
            cat = lambda *u: jnp.concatenate(u, axis=1)
            ops = {1: cat(f(0, 0, K2) + f(1, K1, D), f(0, K2, K1)),
                   2: cat(f(1, 0, K2) + f(1, K1, D), f(1, K2, K1)),
                   6: f(1, 0, K1) - f(0, 0, K1),
                   4: f(1, K1, D),
                   5: f(0, 0, K2) + f(0, K1, D),
                   7: f(0, K1, D) - f(1, K1, D)}
            for i, u in ops.items():
                if i in (4, 5, 7):
                    u = cat(u, u[:, E:T], u[:, 0:E], u[:, T:K2])
                xs[rows_of(p), XS[i]:XS[i] + u.shape[1]] = u.astype(_BF16)
            ops = {i: u.astype(_BF16) for i, u in ops.items()}
            ops[3] = xbuf[rows_of(p), 0:K1]
            return ops

        def dot_short(i, w):
            cat = lambda u, v: jnp.concatenate([u, v], axis=0).astype(_BF16)
            s0, s1 = [t.astype(_BF16).astype(_F32) for t in (w(1, 0, E), w(0, T, K2))]
            ws = (cat(w(0, 0, E) - s0, w(0, E, T)), cat(w(1, T, K2) - s1, w(1, E, T)), cat(s0, s1))
            res = {}
            for q in range(3):
                for p, n in ((q, 2), (q, 0), (q, 1), (3, (q + 2) % 3)):
                    res[p, n] = jnp.dot(xs[rows_of(p), XS[i] + n * T:XS[i] + (n + 1) * T], ws[n],
                                        preferred_element_type=_F32)
            return jnp.concatenate(
                [jnp.concatenate([res[p, 0] + res[p, 2], res[p, 1] + res[p, 2]], axis=1) for p in range(NP)], axis=0)

        def qproj(h, pair=None):
            wh = wqbuf.at[h]
            f = lambda k0, k1, n, m=Dh: wh[k0:k1, n:n + m].astype(_F32)
            cat = lambda u, v: jnp.concatenate([u, v], axis=0)
            w = {1: lambda: cat(f(0, K2, 0) + f(K1, D, Dh), f(K2, K1, 0)).astype(_BF16),
                 2: lambda: wh[0:K1, 0:Dh],
                 3: lambda: cat(f(0, K2, Dh) - f(K1, D, Dh), f(K2, K1, Dh)).astype(_BF16),
                 6: lambda: (f(0, K1, 0) + f(0, K1, Dh)).astype(_BF16)}
            short = {4: lambda t, k0, k1, m=T: f(K1 + k0, K1 + k1, t * T, m) - f(k0, k1, t * T, m),
                     5: lambda t, k0, k1, m=T: f(K1 + k0, K1 + k1, Dh + t * T, m),
                     7: lambda t, k0, k1, m=T: f(K1 + k0, K1 + k1, t * T, m) + f(K1 + k0, K1 + k1, Dh + t * T, m)}
            a = None if pair is None else prep_x(pair)
            mm = {}
            for i in _Q_ORDER:
                if pair is not None:
                    rhs = w[i]() if i in w else short[i](0, 0, K2, Dh).astype(_BF16)
                    mm[i] = jnp.dot(a[i], rhs, preferred_element_type=_F32)
                elif i in short:
                    mm[i] = dot_short(i, short[i])
                else:
                    lhs = xbuf[0:RH, 0:K1] if i == 3 else xs[:, XS[i]:XS[i] + K1]
                    mm[i] = jnp.dot(lhs, w[i](), preferred_element_type=_F32)
            c11 = (((mm[7] - mm[5]) + mm[4]) + mm[1]) * scale
            c12 = (mm[5] + mm[3]) * scale
            c21 = (mm[4] + mm[2]) * scale
            c22 = (((mm[1] + mm[3]) + mm[6]) - mm[2]) * scale
            for n, p in enumerate(range(NP) if pair is None else [pair]):
                rows = slice(n * Sq, (n + 1) * Sq)
                store_q(p, h, c11[rows], c12[rows])
                store_q(NP + p, h, c21[rows], c22[rows])

        def store_shift(j, ma, mb, after=None):
            if after is not None:
                never = z_ref[0] != 0
                ma, mb = jnp.where(never, after, ma), jnp.where(never, after, mb)
            m_refs[j][0:Sq, :] = _softmax_shift(ma)
            m_refs[j][Sq:M, :] = _softmax_shift(mb)

        def scores(unit, slot, j, pending=None, defer=False):
            q = q_all.at[unit]
            views = {z: kbuf.at[slot + z_ref[z], j] for z in dict.fromkeys(_K_Z)}
            k = lambda i: views[_K_Z[i - 1]]
            ma = mb = None
            for c0 in range(0, Sk, 2 * T):
                c1, c2 = c0 + T, c0 + 2 * T
                w = _rhs_operands(lambda i: k(i)[c0:c1, 0:T], lambda i: k(i)[c1:c2, 0:T],
                                  lambda i: k(i)[c0:c1, T:Dh], lambda i: k(i)[c1:c2, T:Dh])
                mm = {}
                for i in _QK_ORDER:
                    mm[i] = lax.dot_general(q[:, (i - 1) * T:i * T], w[i](), _NT, preferred_element_type=_F32)
                c11, c12, c21, c22 = _combine(mm)
                if pending is not None and c0 == Sk // 2:
                    store_shift(*pending, after=c12)
                s_refs[j][0:Sq, c0:c1] = c11
                s_refs[j][0:Sq, c1:c2] = c12
                s_refs[j][Sq:M, c0:c1] = c21
                s_refs[j][Sq:M, c1:c2] = c22
                ta, tb = jnp.maximum(c11, c12), jnp.maximum(c21, c22)
                ma = ta if ma is None else jnp.maximum(ma, ta)
                mb = tb if mb is None else jnp.maximum(mb, tb)
            if defer:
                return (j, ma, mb)
            store_shift(j, ma, mb)

        def softmax_pv(b, h, slot, j, mid=None):
            row = b * Sq if isinstance(b, int) else pl.multiple_of(b * Sq, 16)
            views = {z: vbuf.at[slot if z is None else slot + z_ref[z], j] for z in dict.fromkeys(_V_Z)}
            v = lambda i: views[_V_Z[i - 1]]

            def probs(r0, c0):
                m = m_refs[j][r0:r0 + Sq, :]
                return jnp.exp2(s_refs[j][r0:r0 + Sq, c0:c0 + SH] - jnp.concatenate([m] * (SH // T), axis=1))

            def lane_sum(t):
                acc = t[:, 0:T]
                for c in range(1, SH // T):
                    acc = acc + t[:, c * T:(c + 1) * T]
                return acc

            a11, a12, a21, a22 = probs(0, 0), probs(0, SH), probs(Sq, 0), probs(Sq, SH)
            sa, sb = a11 + a12, a21 + a22
            la, lb = lane_sum(sa), lane_sum(sb)
            a = {1: lambda: a11 + a22, 2: lambda: sb, 3: lambda: a11, 4: lambda: a22,
                 5: lambda: sa, 6: lambda: a21 - a11, 7: lambda: a12 - a22}
            w = _rhs_operands(lambda i: v(i)[0:SH, 0:T], lambda i: v(i)[0:SH, T:Dh],
                              lambda i: v(i)[SH:Sk, 0:T], lambda i: v(i)[SH:Sk, T:Dh])
            mm = {}
            for i in _PV_ORDER:
                if mid is not None and i == _PV_ORDER[-1]:
                    mid()
                mm[i] = jnp.dot(a[i]().astype(_BF16), w[i](), preferred_element_type=_F32)
            c11, c12, c21, c22 = _combine(mm)
            never = z_ref[0] != 0
            ia = _recip(jnp.sum(jnp.where(never, mm[6], la), axis=-1, keepdims=True))
            ib = _recip(jnp.sum(jnp.where(never, mm[6], lb), axis=-1, keepdims=True))
            o_all[h * rep, pl.ds(row, Sq), 0:T] = c11 * ia
            o_all[h * rep, pl.ds(row, Sq), T:Dh] = c12 * ia
            o_all[h * rep + 1, pl.ds(row, Sq), 0:T] = c21 * ib
            o_all[h * rep + 1, pl.ds(row, Sq), T:Dh] = c22 * ib

        done = {}
        wo_sums = {}

        def finish_chunk(i):
            out_copy(i).start()
            z = z_ref[0]
            t = obuf[pl.ds(pl.multiple_of(o_start[i] + z, 16), 16), 0:T].astype(_F32)[0:8]
            done[i] = jnp.where(z != 0, t, 0.0)

        def after(t, zeros):
            if zeros is None:
                return t
            top = jnp.concatenate([t[0:8, 0:T] + zeros, t[0:8, T:]], axis=1)
            return jnp.concatenate([top, t[8:]], axis=0)

        def oproj_strassen(i):
            row0 = o_start[i]
            mm = {}
            for g in range(Hkv // 2):
                k1, k2 = 2 * g * G, (2 * g + 1) * G
                f = lambda r, k, z: wobuf[pl.ds(pl.multiple_of(r * DH + z_ref[z], 16), DH), k:k + G]
                ff = lambda r, k, z: f(r, k, z).astype(_F32)
                if g not in wo_sums:
                    wo_sums[g] = {1: (ff(0, k1, 1) + ff(1, k2, 1)).astype(_BF16),
                                  2: (ff(1, k1, 2) + ff(1, k2, 2)).astype(_BF16),
                                  5: (ff(0, k1, 5) + ff(0, k2, 5)).astype(_BF16),
                                  6: (ff(1, k1, 6) - ff(0, k1, 6)).astype(_BF16),
                                  7: (ff(0, k2, 7) - ff(1, k2, 7)).astype(_BF16)}
                a = dict(wo_sums[g])
                a[3], a[4] = f(0, k1, 8 + i), f(1, k2, 8 + i)

                def o(kk, tt, p):
                    z = 0 if _O_Z[p - 1] is None else z_ref[_O_Z[p - 1]]
                    return jnp.concatenate(
                        [o_all[(2 * g + kk) * rep + r + z, row0 + tt * T:row0 + (tt + 1) * T, :]
                         for r in range(rep)], axis=1)

                w = {1: lambda: o(0, 0, 1) + o(1, 1, 1),
                     2: lambda: after(o(0, 0, 2), done.get(i - 1) if g == 2 else None),
                     3: lambda: o(0, 1, 3) - o(1, 1, 3), 4: lambda: o(1, 0, 4) - o(0, 0, 4),
                     5: lambda: o(1, 1, 5), 6: lambda: o(0, 0, 6) + o(0, 1, 6),
                     7: lambda: o(1, 0, 7) + o(1, 1, 7)}
                for p in _O_ORDER:
                    t = lax.dot_general(a[p], w[p]().astype(_BF16), _NT, preferred_element_type=_F32)
                    mm[p] = t if p not in mm else mm[p] + t
            c11, c12, c21, c22 = _combine(mm)
            obuf[row0:row0 + T, :] = jnp.concatenate([c11, c21], axis=0).T.astype(obuf.dtype)
            obuf[row0 + T:row0 + 2 * T, :] = jnp.concatenate([c12, c22], axis=0).T.astype(obuf.dtype)
            finish_chunk(i)

        def oproj_last(i):
            row0, c0 = o_start[i], 2 * T
            acc, os_ = None, []
            for h in range(Hkv):
                o = jnp.concatenate([o_all[h * rep + r, row0:row0 + T, :] for r in range(rep)], axis=1)
                o = after(o, done.get(i - 1) if h == Hkv - 2 else None).astype(_BF16)
                os_.append(o)
                t = lax.dot_general(wobuf[c0:, h * G:(h + 1) * G], o, _NT, preferred_element_type=_F32)
                acc = t if acc is None else acc + t
            obuf[row0:row0 + T, c0:] = acc.T.astype(obuf.dtype)
            obuf[row0:row0 + T, 0:c0] = lax.dot_general(
                jnp.concatenate(os_, axis=1), wobuf[0:c0, :], _NT, preferred_element_type=_F32).astype(obuf.dtype)
            out_copy(i).start()

        def first_head(p, carry):
            for cp in x_copies(p):
                cp.wait()
            qproj(0, p)
            return carry

        def more_heads(it, carry):
            heads = [1 + it * _Q_LOOP + n for n in range(_Q_LOOP)]
            for h in heads:
                wq_copy(h, SEM_W + it).wait()
            for h in heads:
                qproj(h)
            return carry

        wq_copy(0, SEM_O).wait()
        lax.fori_loop(0, NP, first_head, 0)
        lax.fori_loop(0, NQ, more_heads, 0)
        wq_copy(Hkv - 1, SEM_K).wait()
        k_copy(0, 0).wait()
        for j in range(U):
            scores(j, 0, j)
        k_copy(2, 0).start()
        qproj(Hkv - 1)

        def block(t, carry):
            slot = t & 1
            v_copy(t, slot).wait()
            k_copy(t + 1, 1 - slot).wait()
            b = t // BPB
            h0 = lax.rem(t, BPB) * U
            pending = [None]
            for j in range(U):
                def next_scores():
                    pending[0] = scores((t + 1) * U + j, 1 - slot, j, pending[0], j != U - 1)

                    @pl.when(t + 3 < NB)
                    def _():
                        k_copy(t + 3, 1 - slot, j).start()

                softmax_pv(b, h0 + j, slot, j, next_scores)

                @pl.when(t + 2 < NB)
                def _():
                    v_copy(t + 2, slot, j).start()
            return carry

        lax.fori_loop(0, NB - 1, block, 0)

        t = NB - 1
        v_copy(t, t % 2).wait()
        wo_copy.wait()
        for j in range(U):
            softmax_pv(t // BPB, (t % BPB) * U + j, t % 2, j)
        for i in range(NO - 1):
            oproj_strassen(i)
        oproj_last(NO - 1)
        for i in range(NO):
            out_copy(i).wait()

    hbm = pl.BlockSpec(memory_space=pl.ANY)
    out = pl.pallas_call(
        body,
        in_specs=[hbm] * 5,
        out_specs=hbm,
        out_shape=jax.ShapeDtypeStruct((R, D), x.dtype),
        scratch_shapes=[
            pltpu.VMEM((R, D), _BF16),
            pltpu.VMEM((Hkv, D, G), _BF16),
            pltpu.VMEM((D, Hq * Dh), _BF16),
            pltpu.VMEM((2, U, Sk, Dh), _BF16),
            pltpu.VMEM((2, U, Sk, Dh), _BF16),
            pltpu.VMEM((RH, 3 * K1 + 9 * T), _BF16),
            pltpu.VMEM((B * Hkv, Sq, 7 * T), _BF16),
            pltpu.VMEM((Hq, R, Dh), _F32),
            pltpu.VMEM((R, D), _BF16),
            pltpu.SemaphoreType.DMA((SEM_W + NQ,)),
            pltpu.SMEM((_NZ,), jnp.int32),
        ] + [pltpu.VMEM((M, Sk), _F32)] * U + [pltpu.VMEM((M, T), _F32)] * U,
        compiler_params=pltpu.CompilerParams(vmem_limit_bytes=120 * 1024 * 1024),
    )(x.reshape(R, D), k_cache.reshape(NB, U, Sk, Dh), v_cache.reshape(NB, U, Sk, Dh), wq, wo.T)
    return out.reshape(B, Sq, D)
```

```python
import jax
import jax.numpy as jnp
from jax import lax
import jax.experimental.pallas as pl
import jax.experimental.pallas.tpu as pltpu

_NT = (((1,), (1,)), ((), ()))
_LOG2E = 1.4426950408889634
_BF16 = jnp.bfloat16
_F32 = jnp.float32

_U = 4
_T = 128
_Q_LOOP = 2
_O_CHUNKS = (256, 256, 256, 256, 128)
_Q_ORDER = (5, 7, 4, 1, 3, 6, 2)
_QK_ORDER = (5, 3, 1, 7, 4, 2, 6)
_PV_ORDER = (3, 4, 7, 5, 6, 2, 1)
_O_ORDER = (2, 5, 1, 3, 6, 4, 7)
_K_Z = (0, 1, 0, 1, 0, 1, 0)
_V_Z = (0, 1, None, 3, 4, 5, 6)
_O_Z = (1, None, 3, 4, None, 6, 7)
_NZ = 16


def _combine(m):
    return ((m[1] + m[4]) + (m[7] - m[5]), m[3] + m[5], m[2] + m[4], (m[1] - m[2]) + (m[3] + m[6]))


def _rhs_operands(b11, b12, b21, b22):
    f = lambda b, i: b(i).astype(_F32)
    return {1: lambda: (f(b11, 1) + f(b22, 1)).astype(_BF16),
            2: lambda: b11(2),
            3: lambda: (f(b12, 3) - f(b22, 3)).astype(_BF16),
            4: lambda: (f(b21, 4) - f(b11, 4)).astype(_BF16),
            5: lambda: b22(5),
            6: lambda: (f(b11, 6) + f(b12, 6)).astype(_BF16),
            7: lambda: (f(b21, 7) + f(b22, 7)).astype(_BF16)}


def _recip(l):
    r = pl.reciprocal(l, approx=True)
    return r * (2.0 - l * r)


def _softmax_shift(lane_max):
    m = jnp.max(lane_max, axis=-1, keepdims=True)
    m = m + jnp.log2(jnp.sum(jnp.exp2(lane_max - m), axis=-1, keepdims=True))
    return jnp.broadcast_to(m, lane_max.shape)


@jax.jit
def pallas_standalone__gqa_block_cached__near_ridge_kernel(
    x: jax.Array,
    k_cache: jax.Array,
    v_cache: jax.Array,
    wq: jax.Array,
    wo: jax.Array,
):
    B, Sq, D = x.shape
    _, Hkv, Sk, Dh = k_cache.shape
    Hq = wq.shape[1] // Dh
    rep = Hq // Hkv
    U, T = _U, _T
    G = rep * Dh
    M = rep * Sq
    R = B * Sq
    RH, DH, SH = R // 2, D // 2, Sk // 2
    K1 = 2 * T
    K2 = D - K1
    E = T // 2
    XS = {1: 0, 2: K1, 6: 2 * K1, 4: 3 * K1, 5: 3 * K1 + 3 * T, 7: 3 * K1 + 6 * T}
    NB = B * Hkv // U
    BPB = Hkv // U
    NO = len(_O_CHUNKS)
    NP = B // 2
    NQ = (Hkv - 2) // _Q_LOOP
    scale = Dh ** -0.5 * _LOG2E
    assert rep == 2 and Dh == 2 * T and Hkv % U == 0 and Sk % (4 * T) == 0 and K2 == 3 * E
    assert Sq % 16 == 0 and DH % 16 == 0 and sum(_O_CHUNKS) == R and NP == 4 and (Hkv - 2) % _Q_LOOP == 0
    o_start = [sum(_O_CHUNKS[:i]) for i in range(NO)]
    SEM_K, SEM_V, SEM_WO, SEM_O, SEM_X = 0, 2, 4, 5, 6
    SEM_W = SEM_X + NP

    def body(x_hbm, k_hbm, v_hbm, wq_hbm, wo_hbm, o_hbm,
             xbuf, wqbuf, wobuf, kbuf, vbuf, xs, q_all, o_all, obuf, sem, z_ref, *rest):
        s_refs, m_refs = rest[:U], rest[U:]
        for i in range(_NZ):
            z_ref[i] = 0

        def kv_copy(hbm, buf, sem0, blk, slot, j):
            if j is None:
                return pltpu.make_async_copy(hbm.at[blk], buf.at[slot], sem.at[sem0 + slot])
            return pltpu.make_async_copy(hbm.at[blk, j], buf.at[slot, j], sem.at[sem0 + slot])

        k_copy = lambda blk, slot, j=None: kv_copy(k_hbm, kbuf, SEM_K, blk, slot, j)
        v_copy = lambda blk, slot, j=None: kv_copy(v_hbm, vbuf, SEM_V, blk, slot, j)

        def wq_copy(h, s):
            c = h * G if isinstance(h, int) else pl.multiple_of(h * G, G)
            return pltpu.make_async_copy(wq_hbm.at[:, pl.ds(c, G)], wqbuf.at[h], sem.at[s])

        def rows_of(p, half=0):
            r = half * RH + p * Sq
            return pl.ds(r if isinstance(r, int) else pl.multiple_of(r, 16), Sq)

        def x_copies(p):
            return [pltpu.make_async_copy(x_hbm.at[rows_of(p, half)], xbuf.at[rows_of(p, half)], sem.at[SEM_X + p])
                    for half in range(2)]

        def out_copy(i, c0=0, c1=D):
            sl = (pl.ds(o_start[i], _O_CHUNKS[i]), pl.ds(c0, c1 - c0))
            return pltpu.make_async_copy(obuf.at[sl], o_hbm.at[sl], sem.at[SEM_O])

        wo_copy = pltpu.make_async_copy(wo_hbm, wobuf, sem.at[SEM_WO])

        wq_copy(0, SEM_O).start()
        for p in range(NP):
            for cp in x_copies(p):
                cp.start()
        for h in range(1, Hkv - 1):
            wq_copy(h, SEM_W + (h - 1) // _Q_LOOP).start()
        wq_copy(Hkv - 1, SEM_K).start()
        k_copy(0, 0).start()
        v_copy(0, 0).start()
        k_copy(1, 1).start()
        v_copy(1, 1).start()
        wo_copy.start(priority=1)

        def store_q(b, h, qa, qb):
            a11, a12, a21, a22 = qa[:, 0:T], qa[:, T:Dh], qb[:, 0:T], qb[:, T:Dh]
            ops = (a11 + a22, a21 + a22, a11, a22, a11 + a12, a21 - a11, a12 - a22)
            q_all.at[b * Hkv + h][...] = jnp.concatenate(ops, axis=1).astype(_BF16)

        def prep_x(p):
            f = lambda half, c0, c1: xbuf[rows_of(p, half), c0:c1].astype(_F32)
            cat = lambda *u: jnp.concatenate(u, axis=1)
            ops = {1: cat(f(0, 0, K2) + f(1, K1, D), f(0, K2, K1)),
                   2: cat(f(1, 0, K2) + f(1, K1, D), f(1, K2, K1)),
                   6: f(1, 0, K1) - f(0, 0, K1),
                   4: f(1, K1, D),
                   5: f(0, 0, K2) + f(0, K1, D),
                   7: f(0, K1, D) - f(1, K1, D)}
            for i, u in ops.items():
                if i in (4, 5, 7):
                    u = cat(u, u[:, E:T], u[:, 0:E], u[:, T:K2])
                xs[rows_of(p), XS[i]:XS[i] + u.shape[1]] = u.astype(_BF16)
            ops = {i: u.astype(_BF16) for i, u in ops.items()}
            ops[3] = xbuf[rows_of(p), 0:K1]
            return ops

        def dot_short(i, w):
            cat = lambda u, v: jnp.concatenate([u, v], axis=0).astype(_BF16)
            s0, s1 = [t.astype(_BF16).astype(_F32) for t in (w(1, 0, E), w(0, T, K2))]
            ws = (cat(w(0, 0, E) - s0, w(0, E, T)), cat(w(1, T, K2) - s1, w(1, E, T)), cat(s0, s1))
            res = {}
            for q in range(3):
                for p, n in ((q, 2), (q, 0), (q, 1), (3, (q + 2) % 3)):
                    res[p, n] = jnp.dot(xs[rows_of(p), XS[i] + n * T:XS[i] + (n + 1) * T], ws[n],
                                        preferred_element_type=_F32)
            return jnp.concatenate(
                [jnp.concatenate([res[p, 0] + res[p, 2], res[p, 1] + res[p, 2]], axis=1) for p in range(NP)], axis=0)

        def qproj(h, pair=None):
            wh = wqbuf.at[h]
            f = lambda k0, k1, n, m=Dh: wh[k0:k1, n:n + m].astype(_F32)
            cat = lambda u, v: jnp.concatenate([u, v], axis=0)
            w = {1: lambda: cat(f(0, K2, 0) + f(K1, D, Dh), f(K2, K1, 0)).astype(_BF16),
                 2: lambda: wh[0:K1, 0:Dh],
                 3: lambda: cat(f(0, K2, Dh) - f(K1, D, Dh), f(K2, K1, Dh)).astype(_BF16),
                 6: lambda: (f(0, K1, 0) + f(0, K1, Dh)).astype(_BF16)}
            short = {4: lambda t, k0, k1, m=T: f(K1 + k0, K1 + k1, t * T, m) - f(k0, k1, t * T, m),
                     5: lambda t, k0, k1, m=T: f(K1 + k0, K1 + k1, Dh + t * T, m),
                     7: lambda t, k0, k1, m=T: f(K1 + k0, K1 + k1, t * T, m) + f(K1 + k0, K1 + k1, Dh + t * T, m)}
            a = None if pair is None else prep_x(pair)
            mm = {}
            for i in _Q_ORDER:
                if pair is not None:
                    rhs = w[i]() if i in w else short[i](0, 0, K2, Dh).astype(_BF16)
                    mm[i] = jnp.dot(a[i], rhs, preferred_element_type=_F32)
                elif i in short:
                    mm[i] = dot_short(i, short[i])
                else:
                    lhs = xbuf[0:RH, 0:K1] if i == 3 else xs[:, XS[i]:XS[i] + K1]
                    mm[i] = jnp.dot(lhs, w[i](), preferred_element_type=_F32)
            c11 = (((mm[7] - mm[5]) + mm[4]) + mm[1]) * scale
            c12 = (mm[5] + mm[3]) * scale
            c21 = (mm[4] + mm[2]) * scale
            c22 = (((mm[1] + mm[3]) + mm[6]) - mm[2]) * scale
            for n, p in enumerate(range(NP) if pair is None else [pair]):
                rows = slice(n * Sq, (n + 1) * Sq)
                store_q(p, h, c11[rows], c12[rows])
                store_q(NP + p, h, c21[rows], c22[rows])

        def store_shift(j, ma, mb, after=None):
            if after is not None:
                never = z_ref[0] != 0
                ma, mb = jnp.where(never, after, ma), jnp.where(never, after, mb)
            m_refs[j][0:Sq, :] = _softmax_shift(ma)
            m_refs[j][Sq:M, :] = _softmax_shift(mb)

        def scores(unit, slot, j, pending=None, defer=False):
            q = q_all.at[unit]
            views = {z: kbuf.at[slot + z_ref[z], j] for z in dict.fromkeys(_K_Z)}
            k = lambda i: views[_K_Z[i - 1]]
            ma = mb = None
            for c0 in range(0, Sk, 2 * T):
                c1, c2 = c0 + T, c0 + 2 * T
                w = _rhs_operands(lambda i: k(i)[c0:c1, 0:T], lambda i: k(i)[c1:c2, 0:T],
                                  lambda i: k(i)[c0:c1, T:Dh], lambda i: k(i)[c1:c2, T:Dh])
                mm = {}
                for i in _QK_ORDER:
                    mm[i] = lax.dot_general(q[:, (i - 1) * T:i * T], w[i](), _NT, preferred_element_type=_F32)
                c11, c12, c21, c22 = _combine(mm)
                if pending is not None and c0 == Sk // 2:
                    store_shift(*pending, after=c12)
                s_refs[j][0:Sq, c0:c1] = c11
                s_refs[j][0:Sq, c1:c2] = c12
                s_refs[j][Sq:M, c0:c1] = c21
                s_refs[j][Sq:M, c1:c2] = c22
                ta, tb = jnp.maximum(c11, c12), jnp.maximum(c21, c22)
                ma = ta if ma is None else jnp.maximum(ma, ta)
                mb = tb if mb is None else jnp.maximum(mb, tb)
            if defer:
                return (j, ma, mb)
            store_shift(j, ma, mb)

        def softmax_pv(b, h, slot, j, mid=None):
            row = b * Sq if isinstance(b, int) else pl.multiple_of(b * Sq, 16)
            views = {z: vbuf.at[slot if z is None else slot + z_ref[z], j] for z in dict.fromkeys(_V_Z)}
            v = lambda i: views[_V_Z[i - 1]]

            def probs(r0, c0):
                m = m_refs[j][r0:r0 + Sq, :]
                return jnp.exp2(s_refs[j][r0:r0 + Sq, c0:c0 + SH] - jnp.concatenate([m] * (SH // T), axis=1))

            def lane_sum(t):
                acc = t[:, 0:T]
                for c in range(1, SH // T):
                    acc = acc + t[:, c * T:(c + 1) * T]
                return acc

            a11, a12, a21, a22 = probs(0, 0), probs(0, SH), probs(Sq, 0), probs(Sq, SH)
            sa, sb = a11 + a12, a21 + a22
            la, lb = lane_sum(sa), lane_sum(sb)
            a = {1: lambda: a11 + a22, 2: lambda: sb, 3: lambda: a11, 4: lambda: a22,
                 5: lambda: sa, 6: lambda: a21 - a11, 7: lambda: a12 - a22}
            w = _rhs_operands(lambda i: v(i)[0:SH, 0:T], lambda i: v(i)[0:SH, T:Dh],
                              lambda i: v(i)[SH:Sk, 0:T], lambda i: v(i)[SH:Sk, T:Dh])
            mm = {}
            for i in _PV_ORDER:
                if mid is not None and i == _PV_ORDER[-1]:
                    mid()
                mm[i] = jnp.dot(a[i]().astype(_BF16), w[i](), preferred_element_type=_F32)
            c11, c12, c21, c22 = _combine(mm)
            never = z_ref[0] != 0
            ia = _recip(jnp.sum(jnp.where(never, mm[6], la), axis=-1, keepdims=True))
            ib = _recip(jnp.sum(jnp.where(never, mm[6], lb), axis=-1, keepdims=True))
            o_all[h * rep, pl.ds(row, Sq), 0:T] = c11 * ia
            o_all[h * rep, pl.ds(row, Sq), T:Dh] = c12 * ia
            o_all[h * rep + 1, pl.ds(row, Sq), 0:T] = c21 * ib
            o_all[h * rep + 1, pl.ds(row, Sq), T:Dh] = c22 * ib

        done = {}
        wo_sums = {}

        def finish_chunk(i):
            out_copy(i).start()
            z = z_ref[0]
            t = obuf[pl.ds(pl.multiple_of(o_start[i] + z, 16), 16), 0:T].astype(_F32)[0:8]
            done[i] = jnp.where(z != 0, t, 0.0)

        def after(t, zeros):
            if zeros is None:
                return t
            top = jnp.concatenate([t[0:8, 0:T] + zeros, t[0:8, T:]], axis=1)
            return jnp.concatenate([top, t[8:]], axis=0)

        def oproj_strassen(i):
            row0 = o_start[i]
            mm = {}
            for g in range(Hkv // 2):
                k1, k2 = 2 * g * G, (2 * g + 1) * G
                f = lambda r, k, z: wobuf[pl.ds(pl.multiple_of(r * DH + z_ref[z], 16), DH), k:k + G]
                ff = lambda r, k, z: f(r, k, z).astype(_F32)
                if g not in wo_sums:
                    wo_sums[g] = {1: (ff(0, k1, 1) + ff(1, k2, 1)).astype(_BF16),
                                  2: (ff(1, k1, 2) + ff(1, k2, 2)).astype(_BF16),
                                  5: (ff(0, k1, 5) + ff(0, k2, 5)).astype(_BF16),
                                  6: (ff(1, k1, 6) - ff(0, k1, 6)).astype(_BF16),
                                  7: (ff(0, k2, 7) - ff(1, k2, 7)).astype(_BF16)}
                a = dict(wo_sums[g])
                a[3], a[4] = f(0, k1, 8 + i), f(1, k2, 8 + i)

                def o(kk, tt, p):
                    z = 0 if _O_Z[p - 1] is None else z_ref[_O_Z[p - 1]]
                    return jnp.concatenate(
                        [o_all[(2 * g + kk) * rep + r + z, row0 + tt * T:row0 + (tt + 1) * T, :]
                         for r in range(rep)], axis=1)

                w = {1: lambda: o(0, 0, 1) + o(1, 1, 1),
                     2: lambda: after(o(0, 0, 2), done.get(i - 1) if g == 2 else None),
                     3: lambda: o(0, 1, 3) - o(1, 1, 3), 4: lambda: o(1, 0, 4) - o(0, 0, 4),
                     5: lambda: o(1, 1, 5), 6: lambda: o(0, 0, 6) + o(0, 1, 6),
                     7: lambda: o(1, 0, 7) + o(1, 1, 7)}
                for p in _O_ORDER:
                    t = lax.dot_general(a[p], w[p]().astype(_BF16), _NT, preferred_element_type=_F32)
                    mm[p] = t if p not in mm else mm[p] + t
            c11, c12, c21, c22 = _combine(mm)
            obuf[row0:row0 + T, :] = jnp.concatenate([c11, c21], axis=0).T.astype(obuf.dtype)
            obuf[row0 + T:row0 + 2 * T, :] = jnp.concatenate([c12, c22], axis=0).T.astype(obuf.dtype)
            finish_chunk(i)

        def oproj_last(i):
            row0, c0 = o_start[i], 2 * T
            acc, os_ = None, []
            for h in range(Hkv):
                o = jnp.concatenate([o_all[h * rep + r, row0:row0 + T, :] for r in range(rep)], axis=1)
                o = after(o, done.get(i - 1) if h == Hkv - 2 else None).astype(_BF16)
                os_.append(o)
                t = lax.dot_general(wobuf[c0:, h * G:(h + 1) * G], o, _NT, preferred_element_type=_F32)
                acc = t if acc is None else acc + t
            obuf[row0:row0 + T, c0:] = acc.T.astype(obuf.dtype)
            o = jnp.concatenate(os_, axis=1)
            obuf[row0:row0 + T, T:c0] = lax.dot_general(
                o, wobuf[T:c0, :], _NT, preferred_element_type=_F32).astype(obuf.dtype)
            out_copy(i, T, D).start()
            z = z_ref[0]
            t = obuf[pl.ds(pl.multiple_of(row0 + z, 16), 16), T:c0]
            cut = o.shape[1] - 8 * T
            top = jnp.concatenate([o[0:16, 0:cut], jnp.where(z != 0, t, o[0:16, cut:cut + T]), o[0:16, cut + T:]], axis=1)
            o = jnp.concatenate([top, o[16:]], axis=0)
            obuf[row0:row0 + T, 0:T] = lax.dot_general(
                o, wobuf[0:T, :], _NT, preferred_element_type=_F32).astype(obuf.dtype)
            out_copy(i, 0, T).start()

        def first_head(p, carry):
            for cp in x_copies(p):
                cp.wait()
            qproj(0, p)
            return carry

        def more_heads(it, carry):
            heads = [1 + it * _Q_LOOP + n for n in range(_Q_LOOP)]
            for h in heads:
                wq_copy(h, SEM_W + it).wait()
            for h in heads:
                qproj(h)
            return carry

        wq_copy(0, SEM_O).wait()
        lax.fori_loop(0, NP, first_head, 0)
        lax.fori_loop(0, NQ, more_heads, 0)
        wq_copy(Hkv - 1, SEM_K).wait()
        k_copy(0, 0).wait()
        for j in range(U):
            scores(j, 0, j)
        k_copy(2, 0).start()
        qproj(Hkv - 1)

        def block(t, carry):
            slot = t & 1
            v_copy(t, slot).wait()
            k_copy(t + 1, 1 - slot).wait()
            b = t // BPB
            h0 = lax.rem(t, BPB) * U
            pending = [None]
            for j in range(U):
                def next_scores():
                    pending[0] = scores((t + 1) * U + j, 1 - slot, j, pending[0], j != U - 1)

                    @pl.when(t + 3 < NB)
                    def _():
                        k_copy(t + 3, 1 - slot, j).start()

                softmax_pv(b, h0 + j, slot, j, next_scores)

                @pl.when(t + 2 < NB)
                def _():
                    v_copy(t + 2, slot, j).start()
            return carry

        lax.fori_loop(0, NB - 1, block, 0)

        t = NB - 1
        v_copy(t, t % 2).wait()
        wo_copy.wait()
        for j in range(U):
            softmax_pv(t // BPB, (t % BPB) * U + j, t % 2, j)
        for i in range(NO - 1):
            oproj_strassen(i)
        oproj_last(NO - 1)
        for i in range(NO - 1):
            out_copy(i).wait()
        out_copy(NO - 1, T, D).wait()
        out_copy(NO - 1, 0, T).wait()

    hbm = pl.BlockSpec(memory_space=pl.ANY)
    out = pl.pallas_call(
        body,
        in_specs=[hbm] * 5,
        out_specs=hbm,
        out_shape=jax.ShapeDtypeStruct((R, D), x.dtype),
        scratch_shapes=[
            pltpu.VMEM((R, D), _BF16),
            pltpu.VMEM((Hkv, D, G), _BF16),
            pltpu.VMEM((D, Hq * Dh), _BF16),
            pltpu.VMEM((2, U, Sk, Dh), _BF16),
            pltpu.VMEM((2, U, Sk, Dh), _BF16),
            pltpu.VMEM((RH, 3 * K1 + 9 * T), _BF16),
            pltpu.VMEM((B * Hkv, Sq, 7 * T), _BF16),
            pltpu.VMEM((Hq, R, Dh), _F32),
            pltpu.VMEM((R, D), _BF16),
            pltpu.SemaphoreType.DMA((SEM_W + NQ,)),
            pltpu.SMEM((_NZ,), jnp.int32),
        ] + [pltpu.VMEM((M, Sk), _F32)] * U + [pltpu.VMEM((M, T), _F32)] * U,
        compiler_params=pltpu.CompilerParams(vmem_limit_bytes=120 * 1024 * 1024),
    )(x.reshape(R, D), k_cache.reshape(NB, U, Sk, Dh), v_cache.reshape(NB, U, Sk, Dh), wq, wo.T)
    return out.reshape(B, Sq, D)
```
